```python
import jax
import jax.numpy as jnp

def _softmax(x, axis=-1):
    return jax.nn.softmax(x, axis=axis)
def _gelu(x):
    return jax.nn.gelu(x, approximate=True)
def _silu(x):
    return jax.nn.silu(x)
def _sigmoid(x):
    return jax.nn.sigmoid(x)
def _layernorm(x, axis=-1, eps=1e-5):
    m = jnp.mean(x, axis=axis, keepdims=True)
    v = jnp.var(x, axis=axis, keepdims=True)
    return (x - m) / jnp.sqrt(v + eps)
def _scatter_add(tgt, idx, src, axis=0):
    return tgt.at[idx].add(src)
def _segment_sum(src, seg, n):
    return jax.ops.segment_sum(src, seg, n)
class _Rng:
    def __init__(self, key):
        self._k = key
    def _next(self):
        self._k, sub = jax.random.split(self._k)
        return sub
    def normal(self, shape):
        return jax.random.normal(self._next(), shape, dtype=jnp.bfloat16)
    def randint(self, lo, hi, shape):
        return jax.random.randint(self._next(), shape, lo, hi, dtype=jnp.int32)
    def uniform(self, shape, lo=0.0, hi=1.0):
        return jax.random.uniform(self._next(), shape, jnp.bfloat16, lo, hi)
    def permutation(self, n):
        return jax.random.permutation(self._next(), n)


kernel_name = 'recurrent_scan__sliding_block_cached__mixer_s_mlp__decode'

def setup_inputs():
    _rng = _Rng(jax.random.key(int.from_bytes(__import__("os").urandom(4), "little")))
    _w = (lambda a: (lambda t: t.astype(jnp.bfloat16) if jnp.issubdtype(t.dtype, jnp.floating) else t)(jnp.asarray(a)))
    def _A_setup():
        B, Sq, D = 1, 1, 512
        Hq, Hkv, Sk, Dh = 32, 32, 32768, 128
        assert Hq % Hkv == 0, (Hq, Hkv)
        return {
            "x": _w((lambda *s: _rng.normal(s) * 0.05)(B, Sq, D)),
            "k_cache": _w((lambda *s: _rng.normal(s) * 0.05)(B, Hkv, Sk, Dh)),
            "v_cache": _w((lambda *s: _rng.normal(s) * 0.05)(B, Hkv, Sk, Dh)),
            "wq": _w((lambda *s: _rng.normal(s) * 0.05)(D, Hq * Dh) * (D ** -0.5)),
            "wo": _w((lambda *s: _rng.normal(s) * 0.05)(Hq * Dh, D) * ((Hq * Dh) ** -0.5)),
        }
    _A_in = _A_setup()

    def _B_setup():
        B, S, D, F = 1, 1, 512, 1376
        return {
            "x":  _w((lambda *s: _rng.normal(s) * 0.05)(B, S, D)),
            "w1": _w((lambda *s: _rng.normal(s) * 0.05)(D, D) * (D ** -0.5)),
            "w2": _w((lambda *s: _rng.normal(s) * 0.05)(D, D) * (D ** -0.5)),
            "w3": _w((lambda *s: _rng.normal(s) * 0.05)(D, F) * (D ** -0.5)),
            "w4": _w((lambda *s: _rng.normal(s) * 0.05)(F, D) * (F ** -0.5)),
        }
    _B_in = _B_setup()

    return {
        "A_x": _A_in["x"],
        "A_k_cache": _A_in["k_cache"],
        "A_v_cache": _A_in["v_cache"],
        "A_wq": _A_in["wq"],
        "A_wo": _A_in["wo"],
        "B_x": _B_in["x"],
        "B_w1": _B_in["w1"],
        "B_w2": _B_in["w2"],
        "B_w3": _B_in["w3"],
        "B_w4": _B_in["w4"],
    }

def reference(A_x, A_k_cache, A_v_cache, A_wq, A_wo, B_x, B_w1, B_w2, B_w3, B_w4):
    def _A_ref(x, k_cache, v_cache, wq, wo):
        B, Sq, D = x.shape
        Hq, Dh = 32, 128
        Hkv, Sk = k_cache.shape[1], k_cache.shape[2]
        W = min(4096, max(256, Sk // 4))
        rep = Hq // Hkv
        q = (lambda x, *d: x.transpose(*d))((x @ wq).reshape(B, Sq, Hq, Dh), 0, 2, 1, 3)
        k = jnp.repeat(k_cache[:, :, Sk - W:, :], rep, axis=1)
        v = jnp.repeat(v_cache[:, :, Sk - W:, :], rep, axis=1)
        scores = jnp.einsum("bhqd,bhkd->bhqk", q, k) * (Dh ** -0.5)
        p = _softmax(scores, axis=-1)
        o = jnp.einsum("bhqk,bhkd->bhqd", p, v)
        return (lambda x, *d: x.transpose(*d))(o, 0, 2, 1, 3).reshape(B, Sq, Hq * Dh) @ wo

    def _B_ref(x, w1, w2, w3, w4):
        B, S, D = x.shape
        h = _gelu(_layernorm(x, axis=-1) @ w1)
        c = D // 4
        g0 = jnp.pad(h[:, :, 0*c:1*c], ((0, 0), (1, 0), (0, 0)))[:, :S, :]
        g1 = jnp.pad(h[:, :, 1*c:2*c], ((0, 0), (0, 1), (0, 0)))[:, 1:, :]
        g2 = jnp.pad(h[:, :, 2*c:3*c], ((0, 0), (2, 0), (0, 0)))[:, :S, :]
        g3 = jnp.pad(h[:, :, 3*c:   ], ((0, 0), (0, 2), (0, 0)))[:, 2:, :]
        hs = jnp.concatenate([g0, g1, g2, g3], axis=-1) @ w2
        x1 = x + hs
        h2 = _gelu(_layernorm(x1, axis=-1) @ w3) @ w4
        return x1 + h2

    x = A_x
    xn = _layernorm(x, axis=-1)
    s = _A_ref(xn, A_k_cache, A_v_cache, A_wq, A_wo)
    g = _silu(_B_ref(xn, B_w1, B_w2, B_w3, B_w4))
    return x + s * g
```

```python
import functools

import jax
import jax.numpy as jnp
import jax.experimental.pallas as pl
import jax.experimental.pallas.tpu as pltpu

_EPS = 1e-5
F32 = jnp.float32
BF16 = jnp.bfloat16
NT = (((1,), (1,)), ((), ()))


def _layernorm(x):
    m = jnp.mean(x, axis=-1, keepdims=True)
    xc = x - m
    v = jnp.mean(xc * xc, axis=-1, keepdims=True)
    return xc / jnp.sqrt(v + _EPS)


def _split_units(total_units, n):
    base, rem = divmod(total_units, n)
    return [base + (1 if i < rem else 0) for i in range(n)]


def build(KCH=1024, WP=4, WQCH=32, TAIL=(256, 96), compute=True, debug=False, nobounds=True,
          QSPLIT=4, pin=0, pbulk=1):
    def _kernel(x_hbm, wq_hbm, k_hbm, v_hbm, wo_hbm, w3_hbm, w4_hbm, o_ref, *rest,
                H, W, Sk, Dh, D, F, scale):
        if debug:
            dbg_ref, rest = rest[0], rest[1:]
        (x_v, wq_v, k_v, v_v, wo_v, w3_v, w4_v, q_ref, acc_ref, t_ref,
         sem_x, sem_b, sem_i) = rest
        NC = W // KCH
        PH = 2 * NC
        base = Sk - W
        WOP = Dh // PH

        pro_bulk = []
        for r in range(0, D, WQCH):
            pro_bulk.append((wq_hbm.at[pl.ds(r, WQCH), :], wq_v.at[pl.ds(r, WQCH), :]))
        n_wq = len(pro_bulk)
        w4_early = F - sum(TAIL)
        w4_rows = []
        r = 0
        while r < w4_early:
            n = min(256, w4_early - r)
            pro_bulk.append((w4_hbm.at[pl.ds(r, n), :], w4_v.at[pl.ds(r, n), :]))
            w4_rows.append((r, n))
            r += n
        P = len(pro_bulk)
        pro_inj = []
        r = 0
        for u in _split_units(F // 16, P):
            n = u * 16
            pro_inj.append((w3_hbm.at[pl.ds(r, n), :], w3_v.at[pl.ds(r, n), :]))
            r += n
        tail_bulk = []
        tail_rows = []
        r = w4_early
        for n in TAIL:
            tail_bulk.append((w4_hbm.at[pl.ds(r, n), :], w4_v.at[pl.ds(r, n), :]))
            tail_rows.append((r, n))
            r += n
        T = len(tail_bulk)
        NP = P + H * PH + T

        def head_bulk(h, c):
            if c < NC:
                return (k_hbm.at[0, h, pl.ds(base + c * KCH, KCH), :], k_v.at[h, pl.ds(c * KCH, KCH), :])
            c -= NC
            return (v_hbm.at[0, h, pl.ds(base + c * KCH, KCH), :], v_v.at[h, pl.ds(c * KCH, KCH), :])

        def head_inj(h, c):
            r = h * Dh + c * WOP
            if not isinstance(h, int):
                r = pl.multiple_of(r, WOP)
            return (wo_hbm.at[pl.ds(r, WOP), :], wo_v.at[h, pl.ds(c * WOP, WOP), :])

        assert PH % WP == 0

        def slot_of(lin):
            return lin % WP

        def copies(kind, h, c):
            if kind == 'pro':
                s = slot_of(c)
                bi, ii = pro_bulk[c], pro_inj[c]
            elif kind == 'head':
                s = slot_of(P + c)
                bi, ii = head_bulk(h, c), head_inj(h, c)
            else:
                s = slot_of(P + c)
                bi, ii = tail_bulk[c], None
            b = pltpu.make_async_copy(bi[0], bi[1], sem_b.at[s])
            i = None if ii is None else pltpu.make_async_copy(ii[0], ii[1], sem_i.at[s])
            return i, b

        def lin_copies(lin):
            if lin < P:
                return copies('pro', None, lin)
            if lin < P + H * PH:
                hh, c = divmod(lin - P, PH)
                return copies('head', hh, c)
            if lin < NP:
                return copies('tail', None, lin - P - H * PH)
            return None

        def start(cp):
            if cp is None:
                return
            i, b = cp
            if i is not None:
                i.start(priority=pin)
            b.start(priority=pbulk)

        def wait(cp):
            i, b = cp
            if i is not None:
                i.wait()
            b.wait()

        xcp = pltpu.make_async_copy(x_hbm, x_v, sem_x.at[0])
        xcp.start()
        for i in range(WP):
            start(lin_copies(i))
        xcp.wait()
        x = x_v[0].astype(F32)
        xn = _layernorm(x)
        xn8 = jnp.broadcast_to(xn, (8, D))
        xb = xn8.astype(BF16)
        q = None
        per = n_wq // QSPLIT
        for i in range(P):
            wait(lin_copies(i))
            start(lin_copies(i + WP))
            if compute and i < n_wq and (i + 1) % per == 0:
                r0 = (i + 1 - per) * WQCH
                r1 = (i + 1) * WQCH
                part = jnp.dot(xb[:, r0:r1], wq_v[r0:r1, :], preferred_element_type=F32)
                q = part if q is None else q + part
                if i == n_wq - 1:
                    for hh in range(H):
                        q_ref[hh] = q[:, hh * Dh:(hh + 1) * Dh].astype(BF16)
        if compute:
            y = _layernorm(xn8)
            t = jax.lax.dot_general(y.astype(BF16), w3_v[...], NT, preferred_element_type=F32)
            t = jax.nn.gelu(t, approximate=True).astype(BF16)
            t_ref[...] = t
            h2 = jnp.dot(t[:, :w4_early], w4_v[0:w4_early, :], preferred_element_type=F32)
            acc_ref[0] = jnp.zeros((8, D), F32)
            acc_ref[1] = h2

        def head_body(h, starter):
            s_parts = []
            if compute:
                qh = q_ref[h]
            for c in range(NC):
                wait(copies('head', h, c))
                starter(c)
                if compute:
                    s_parts.append(jax.lax.dot_general(
                        qh, k_v[h, pl.ds(c * KCH, KCH), :], NT, preferred_element_type=F32))
            if compute:
                m = functools.reduce(jnp.maximum, [jnp.max(s, axis=-1, keepdims=True) for s in s_parts])
                p_parts = [jnp.exp((s - m) * scale) for s in s_parts]
                l = functools.reduce(jnp.add, [jnp.sum(p, axis=-1, keepdims=True) for p in p_parts])
                p_parts = [p.astype(BF16) for p in p_parts]
            o = jnp.zeros((8, Dh), F32)
            for c in range(NC):
                wait(copies('head', h, NC + c))
                starter(NC + c)
                if compute:
                    o = o + jnp.dot(p_parts[c], v_v[h, pl.ds(c * KCH, KCH), :],
                                    preferred_element_type=F32)
            if compute:
                o = o / l
                acc_ref[0] += jnp.dot(o.astype(BF16), wo_v[h], preferred_element_type=F32)

        LAc = -(-WP // PH)

        def loop_starter(h, c):
            dh, cc = divmod(c + WP, PH)
            start(copies('head', h + dh, cc))

        def loop_body(h, carry):
            head_body(h, lambda c: loop_starter(h, c))
            return carry

        jax.lax.fori_loop(0, H - LAc, loop_body, 0)
        for hh in range(H - LAc, H):
            head_body(hh, lambda c, hh=hh: start(lin_copies(P + hh * PH + c + WP)))

        for lin in range(P + H * PH + WP, NP):
            start(lin_copies(lin))
        if compute:
            h2 = acc_ref[1]
        for e, (r, n) in enumerate(tail_rows):
            wait(copies('tail', None, e))
            if compute:
                h2 = h2 + jnp.dot(t_ref[:, r:r + n], w4_v[r:r + n, :], preferred_element_type=F32)
        if compute:
            z = xn8 + h2
            g = z * jax.nn.sigmoid(z)
            s = acc_ref[0]
            out = x + (s * g)[0:1]
            o_ref[0] = out.astype(o_ref.dtype)
            if debug:
                dbg_ref[0:8, :] = s
                dbg_ref[8:16, :] = g
        else:
            o_ref[0] = x.astype(o_ref.dtype)
            if debug:
                dbg_ref[...] = jnp.zeros_like(dbg_ref)

    @jax.jit
    def fn(A_x, A_k_cache, A_v_cache, A_wq, A_wo, B_x, B_w1, B_w2, B_w3, B_w4):
        B, Sq, D = A_x.shape
        _, H, Sk, Dh = A_k_cache.shape
        F = B_w3.shape[1]
        W = min(4096, max(256, Sk // 4))
        out_shape = [jax.ShapeDtypeStruct((B, Sq, D), A_x.dtype)]
        out_specs = [pl.BlockSpec(memory_space=pltpu.VMEM)]
        if debug:
            out_shape.append(jax.ShapeDtypeStruct((16, D), F32))
            out_specs.append(pl.BlockSpec(memory_space=pltpu.VMEM))
        res = pl.pallas_call(
            functools.partial(_kernel, H=H, W=W, Sk=Sk, Dh=Dh, D=D, F=F, scale=Dh ** -0.5),
            in_specs=[pl.BlockSpec(memory_space=pl.ANY)] * 7,
            out_specs=out_specs,
            out_shape=out_shape,
            scratch_shapes=[
                pltpu.VMEM((1, 1, D), BF16),
                pltpu.VMEM((D, H * Dh), BF16),
                pltpu.VMEM((H, W, Dh), BF16),
                pltpu.VMEM((H, W, Dh), BF16),
                pltpu.VMEM((H, Dh, D), BF16),
                pltpu.VMEM((F, D), BF16),
                pltpu.VMEM((F, D), BF16),
                pltpu.VMEM((H, 8, Dh), BF16),
                pltpu.VMEM((2, 8, D), F32),
                pltpu.VMEM((8, F), BF16),
                pltpu.SemaphoreType.DMA((1,)),
                pltpu.SemaphoreType.DMA((WP,)),
                pltpu.SemaphoreType.DMA((WP,)),
            ],
            compiler_params=pltpu.CompilerParams(
                vmem_limit_bytes=100 * 1024 * 1024,
                disable_bounds_checks=nobounds,
            ),
        )(A_x, A_wq, A_k_cache, A_v_cache, A_wo, B_w3.T, B_w4)
        return res if debug else res[0]
    return fn

pallas_recurrent_scan__sliding_block_cached__mixer_s_mlp__decode_kernel = build()
```

```python
import functools

import jax
import jax.numpy as jnp
import jax.experimental.pallas as pl
import jax.experimental.pallas.tpu as pltpu

_EPS = 1e-5
_F32 = jnp.float32
_BF16 = jnp.bfloat16
_NT = (((1,), (1,)), ((), ()))

_ROWS = 8
_KV_ROWS = 1024
_WQ_ROWS = 32
_W4_ROWS = 256
_IN_FLIGHT = 4
_DEFERRED = 3
_Q_STEPS = 4
_BULK_PRIO = 1
_SMALL_PRIO = 0


def _layernorm(x):
    m = jnp.mean(x, axis=-1, keepdims=True)
    xc = x - m
    v = jnp.mean(xc * xc, axis=-1, keepdims=True)
    return xc / jnp.sqrt(v + _EPS)


def _kernel(x_hbm, wq_hbm, k_hbm, v_hbm, wo_hbm, w3t_hbm, w4_hbm, out_ref,
            x_v, wq_v, k_v, v_v, wo_v, w3t_v, w4_v, q_v, t_v, o_v, vec_v,
            *, heads, window, seq, dh, d, f):
    scale = dh ** -0.5
    chunks = window // _KV_ROWS
    pairs = 2 * chunks
    small = dh // pairs
    first_key = seq - window
    w4_early = f - _DEFERRED * dh

    pro_bulk = [(wq_hbm, wq_v, r, _WQ_ROWS) for r in range(0, d, _WQ_ROWS)]
    n_wq = len(pro_bulk)
    pro_bulk += [(w4_hbm, w4_v, r, min(_W4_ROWS, w4_early - r))
                 for r in range(0, w4_early, _W4_ROWS)]
    n_pro = len(pro_bulk)
    units, extra = divmod(f // 16, n_pro)
    pro_small, r = [], 0
    for i in range(n_pro):
        n = 16 * (units + (i < extra))
        pro_small.append((w3t_hbm, w3t_v, r, n))
        r += n
    n_stream = n_pro + heads * pairs + _DEFERRED

    def body(sem_x, sem_pro_bulk, sem_pro_small, sem_bulk, sem_small, sem_tail):
        def rows_copy(src, dst, r, n, sem):
            return pltpu.make_async_copy(src.at[pl.ds(r, n), :], dst.at[pl.ds(r, n), :], sem)

        def pro_pair(i):
            return (rows_copy(*pro_small[i], sem_pro_small.at[i]),
                    rows_copy(*pro_bulk[i], sem_pro_bulk.at[i]))

        def head_pair(h, c):
            static = isinstance(h, int)
            if static and h < _DEFERRED:
                sm = rows_copy(w4_hbm, w4_v, w4_early + h * dh + c * small, small,
                               sem_small.at[c])
            else:
                r = h * dh + c * small
                r = r if static else pl.multiple_of(r, small)
                sm = rows_copy(wo_hbm, wo_v, r, small, sem_small.at[c])
            src, dst, j = (k_hbm, k_v, c) if c < chunks else (v_hbm, v_v, c - chunks)
            bulk = pltpu.make_async_copy(
                src.at[0, h, pl.ds(first_key + j * _KV_ROWS, _KV_ROWS), :],
                dst.at[h % 2, pl.ds(j * _KV_ROWS, _KV_ROWS), :],
                sem_bulk.at[c])
            return sm, bulk

        def tail_copy(i):
            return rows_copy(wo_hbm, wo_v, i * dh, dh, sem_tail.at[i])

        def start_pair(pair):
            pair[0].start(priority=_SMALL_PRIO)
            pair[1].start(priority=_BULK_PRIO)

        def wait_pair(pair):
            pair[0].wait()
            pair[1].wait()

        def start_stream(i):
            if i < n_pro:
                start_pair(pro_pair(i))
            elif i < n_pro + heads * pairs:
                start_pair(head_pair(*divmod(i - n_pro, pairs)))
            elif i < n_stream:
                tail_copy(i - n_pro - heads * pairs).start(priority=_BULK_PRIO)

        x_copy = pltpu.make_async_copy(x_hbm, x_v, sem_x.at[0])
        x_copy.start()
        for i in range(_IN_FLIGHT):
            start_stream(i)
        x_copy.wait()
        x = jnp.broadcast_to(x_v[0].astype(_F32), (_ROWS, d))
        xn = _layernorm(x)
        xn_b = xn.astype(_BF16)
        vec_v[0] = x
        vec_v[1] = xn
        vec_v[2] = jnp.zeros((_ROWS, d), _F32)

        q = None
        per_step = n_wq // _Q_STEPS
        for i in range(n_pro):
            wait_pair(pro_pair(i))
            start_stream(i + _IN_FLIGHT)
            if i < n_wq and (i + 1) % per_step == 0:
                r0, r1 = (i + 1 - per_step) * _WQ_ROWS, (i + 1) * _WQ_ROWS
                part = jnp.dot(xn_b[:, r0:r1], wq_v[r0:r1, :], preferred_element_type=_F32)
                q = part if q is None else q + part
                if i == n_wq - 1:
                    for h in range(heads):
                        q_v[h] = q[:, h * dh:(h + 1) * dh].astype(_BF16)
        hidden = jax.lax.dot_general(_layernorm(xn).astype(_BF16), w3t_v[...], _NT,
                                     preferred_element_type=_F32)
        t_v[...] = jax.nn.gelu(hidden, approximate=True).astype(_BF16)

        def head(h, start_ahead):
            qh = q_v[h]
            scores = []
            for c in range(chunks):
                wait_pair(head_pair(h, c))
                start_ahead(c)
                scores.append(jax.lax.dot_general(
                    qh, k_v[h % 2, pl.ds(c * _KV_ROWS, _KV_ROWS), :], _NT,
                    preferred_element_type=_F32))
            m = functools.reduce(
                jnp.maximum, [jnp.max(s, axis=-1, keepdims=True) for s in scores])
            p = [jnp.exp((s - m) * scale) for s in scores]
            l = functools.reduce(jnp.add, [jnp.sum(e, axis=-1, keepdims=True) for e in p])
            o = jnp.zeros((_ROWS, dh), _F32)
            for c in range(chunks):
                wait_pair(head_pair(h, chunks + c))
                start_ahead(chunks + c)
                o = o + jnp.dot(p[c].astype(_BF16),
                                v_v[h % 2, pl.ds(c * _KV_ROWS, _KV_ROWS), :],
                                preferred_element_type=_F32)
            o = (o / l).astype(_BF16)
            if isinstance(h, int) and h < _DEFERRED:
                o_v[h] = o
            else:
                r = h * dh if isinstance(h, int) else pl.multiple_of(h * dh, dh)
                vec_v[2] += jnp.dot(o, wo_v[pl.ds(r, dh), :], preferred_element_type=_F32)

        def static_head(h):
            head(h, lambda c: start_stream(n_pro + h * pairs + c + _IN_FLIGHT))

        for h in range(_DEFERRED):
            static_head(h)

        z = vec_v[1] + jnp.dot(t_v[...], w4_v[...], preferred_element_type=_F32)
        vec_v[3] = z * jax.nn.sigmoid(z)

        def loop_head(h, carry):
            def start_ahead(c):
                dh_, c_ = divmod(c + _IN_FLIGHT, pairs)
                start_pair(head_pair(h + dh_, c_))
            head(h, start_ahead)
            return carry

        jax.lax.fori_loop(_DEFERRED, heads - 1, loop_head, 0)
        static_head(heads - 1)

        s = vec_v[2]
        for i in range(_DEFERRED):
            tail_copy(i).wait()
            s = s + jnp.dot(o_v[i], wo_v[i * dh:(i + 1) * dh, :], preferred_element_type=_F32)
        out = vec_v[0] + s * vec_v[3]
        out_ref[0] = out[0:1].astype(out_ref.dtype)

    dma = pltpu.SemaphoreType.DMA
    pl.run_scoped(body, dma((1,)), dma((n_pro,)), dma((n_pro,)),
                  dma((pairs,)), dma((pairs,)), dma((_DEFERRED,)))


@jax.jit
def pallas_recurrent_scan__sliding_block_cached__mixer_s_mlp__decode_kernel(
    A_x, A_k_cache, A_v_cache, A_wq, A_wo, B_x, B_w1, B_w2, B_w3, B_w4,
):
    b, sq, d = A_x.shape
    _, heads, seq, dh = A_k_cache.shape
    f = B_w3.shape[1]
    window = min(4096, max(256, seq // 4))
    assert b == 1 and sq == 1 and A_wq.shape[1] == heads * dh
    assert window % _KV_ROWS == 0 and _IN_FLIGHT <= 2 * window // _KV_ROWS
    assert _DEFERRED <= _IN_FLIGHT and f % 16 == 0

    return pl.pallas_call(
        functools.partial(_kernel, heads=heads, window=window, seq=seq, dh=dh, d=d, f=f),
        in_specs=[pl.BlockSpec(memory_space=pl.ANY)] * 7,
        out_specs=pl.BlockSpec(memory_space=pltpu.VMEM),
        out_shape=jax.ShapeDtypeStruct((b, sq, d), A_x.dtype),
        scratch_shapes=[
            pltpu.VMEM((1, 1, d), _BF16),
            pltpu.VMEM((d, heads * dh), _BF16),
            pltpu.VMEM((2, window, dh), _BF16),
            pltpu.VMEM((2, window, dh), _BF16),
            pltpu.VMEM((heads * dh, d), _BF16),
            pltpu.VMEM((f, d), _BF16),
            pltpu.VMEM((f, d), _BF16),
            pltpu.VMEM((heads, _ROWS, dh), _BF16),
            pltpu.VMEM((_ROWS, f), _BF16),
            pltpu.VMEM((_DEFERRED, _ROWS, dh), _BF16),
            pltpu.VMEM((4, _ROWS, d), _F32),
        ],
        compiler_params=pltpu.CompilerParams(vmem_limit_bytes=32 * 1024 * 1024),
    )(A_x, A_wq, A_k_cache, A_v_cache, A_wo, B_w3.T, B_w4)
```

```python
import functools

import jax
import jax.numpy as jnp
import jax.experimental.pallas as pl
import jax.experimental.pallas.tpu as pltpu

_EPS = 1e-5
_F32 = jnp.float32
_BF16 = jnp.bfloat16
_NT = (((1,), (1,)), ((), ()))

_ROWS = 8
_KV_ROWS = 256
_KV_HI = 56
_WQ_ROWS = 8
_WQ_HI = 1024
_W_ROWS = 64
_W_HI = 16
_WO_PIECES = 8
_CHUNK = 1024
_AHEAD = 29
_DEFERRED = 3
_TAIL_GAP = 2
_Q_STEPS = 4
_HI, _LO = 0, 1


def _layernorm(x):
    m = jnp.mean(x, axis=-1, keepdims=True)
    xc = x - m
    v = jnp.mean(xc * xc, axis=-1, keepdims=True)
    return xc / jnp.sqrt(v + _EPS)


def _kernel(x_hbm, wq_hbm, k_hbm, v_hbm, wo_hbm, w3t_hbm, w4_hbm, out_ref,
            x_v, wq_v, k_v, v_v, wo_v, w3t_v, w4_v, q_v, t_v, o_v, vec_v,
            *, heads, window, seq, dh, d, f):
    scale = dh ** -0.5
    n_pos = window // _KV_ROWS
    per_head = 2 * n_pos
    per_chunk = _CHUNK // _KV_ROWS
    chunks = window // _CHUNK
    piece = dh // _WO_PIECES
    every = per_head // _WO_PIECES
    first_key = seq - window
    w4_early = f - _DEFERRED * dh
    all_cols = slice(None)

    pro = [((wq_hbm, wq_v, pl.ds(r, _WQ_ROWS), pl.ds(0, _WQ_HI)),
            (wq_hbm, wq_v, pl.ds(r, _WQ_ROWS), pl.ds(_WQ_HI, heads * dh - _WQ_HI)))
           for r in range(0, d, _WQ_ROWS)]
    n_wq = len(pro)
    for src, dst, total in ((w3t_hbm, w3t_v, f), (w4_hbm, w4_v, w4_early)):
        for r in range(0, total, _W_ROWS):
            n = min(_W_ROWS, total - r)
            if n > _W_HI:
                pro.append(((src, dst, pl.ds(r, _W_HI), all_cols),
                            (src, dst, pl.ds(r + _W_HI, n - _W_HI), all_cols)))
            else:
                pro.append((None, (src, dst, pl.ds(r, n), all_cols)))
    n_pro = len(pro)
    n_el = n_pro + heads * per_head

    def body(sem_x, sem_pro_hi, sem_pro_lo, sem_hi, sem_lo, sem_piece, sem_tail):
        def block_copy(spec, sem):
            src, dst, rows, cols = spec
            return pltpu.make_async_copy(src.at[rows, cols], dst.at[rows, cols], sem)

        def pro_el(i):
            hi, lo = pro[i]
            his = [] if hi is None else [functools.partial(block_copy, hi, sem_pro_hi.at[i])]
            return his, functools.partial(block_copy, lo, sem_pro_lo.at[i])

        def head_el(h, c):
            static = isinstance(h, int)
            his = []
            if c % every == 0:
                w = c // every
                if static and h < _DEFERRED:
                    rows = pl.ds(w4_early + h * dh + w * piece, piece)
                    spec = (w4_hbm, w4_v, rows, all_cols)
                else:
                    r = h * dh + w * piece
                    r = r if static else pl.multiple_of(r, piece)
                    spec = (wo_hbm, wo_v, pl.ds(r, piece), all_cols)
                his.append(functools.partial(block_copy, spec, sem_piece.at[w]))
            src, dst, j = (k_hbm, k_v, c) if c < n_pos else (v_hbm, v_v, c - n_pos)

            def kv_copy(r, n, sem):
                return pltpu.make_async_copy(src.at[0, h, pl.ds(first_key + r, n), :],
                                             dst.at[h % 2, pl.ds(r, n), :], sem)

            his.append(functools.partial(kv_copy, j * _KV_ROWS, _KV_HI, sem_hi.at[c]))
            lo = functools.partial(kv_copy, j * _KV_ROWS + _KV_HI, _KV_ROWS - _KV_HI,
                                   sem_lo.at[c])
            return his, lo

        def element(i):
            return pro_el(i) if i < n_pro else head_el(*divmod(i - n_pro, per_head))

        def tail_copy(i):
            return block_copy((wo_hbm, wo_v, pl.ds(i * dh, dh), all_cols), sem_tail.at[i])

        def start_el(el):
            for cp in el[0]:
                cp().start(priority=_HI)
            el[1]().start(priority=_LO)

        def wait_el(el):
            for cp in el[0]:
                cp().wait()
            el[1]().wait()

        def advance(i):
            j = i + _AHEAD
            if j < n_el:
                start_el(element(j))
            elif (j - n_el) % _TAIL_GAP == 0 and (j - n_el) // _TAIL_GAP < _DEFERRED:
                tail_copy((j - n_el) // _TAIL_GAP).start(priority=_LO)

        x_copy = pltpu.make_async_copy(x_hbm, x_v, sem_x.at[0])
        x_copy.start()
        for i in range(_AHEAD):
            start_el(element(i))
        x_copy.wait()
        x = jnp.broadcast_to(x_v[0].astype(_F32), (_ROWS, d))
        xn = _layernorm(x)
        xn_b = xn.astype(_BF16)
        vec_v[0] = x
        vec_v[1] = xn
        vec_v[2] = jnp.zeros((_ROWS, d), _F32)

        q = None
        per_step = n_wq // _Q_STEPS
        for i in range(n_pro):
            wait_el(element(i))
            advance(i)
            if i < n_wq and (i + 1) % per_step == 0:
                r1 = (i + 1) * _WQ_ROWS
                r0 = r1 - per_step * _WQ_ROWS
                part = jnp.dot(xn_b[:, r0:r1], wq_v[r0:r1, :], preferred_element_type=_F32)
                q = part if q is None else q + part
                if i == n_wq - 1:
                    for h in range(heads):
                        q_v[h] = q[:, h * dh:(h + 1) * dh].astype(_BF16)
        hidden = jax.lax.dot_general(_layernorm(xn).astype(_BF16), w3t_v[...], _NT,
                                     preferred_element_type=_F32)
        t_v[...] = jax.nn.gelu(hidden, approximate=True).astype(_BF16)

        def head(h, advance_from):
            def arrive(first):
                for c in range(first, first + per_chunk):
                    wait_el(head_el(h, c))
                    advance_from(c)

            qh = q_v[h]
            scores = []
            for c in range(chunks):
                arrive(c * per_chunk)
                scores.append(jax.lax.dot_general(
                    qh, k_v[h % 2, pl.ds(c * _CHUNK, _CHUNK), :], _NT,
                    preferred_element_type=_F32))
            m = functools.reduce(
                jnp.maximum, [jnp.max(s, axis=-1, keepdims=True) for s in scores])
            p = [jnp.exp((s - m) * scale) for s in scores]
            l = functools.reduce(jnp.add, [jnp.sum(e, axis=-1, keepdims=True) for e in p])
            o = jnp.zeros((_ROWS, dh), _F32)
            for c in range(chunks):
                arrive(n_pos + c * per_chunk)
                o = o + jnp.dot(p[c].astype(_BF16),
                                v_v[h % 2, pl.ds(c * _CHUNK, _CHUNK), :],
                                preferred_element_type=_F32)
            o = (o / l).astype(_BF16)
            if isinstance(h, int) and h < _DEFERRED:
                o_v[h] = o
            else:
                r = h * dh if isinstance(h, int) else pl.multiple_of(h * dh, dh)
                vec_v[2] += jnp.dot(o, wo_v[pl.ds(r, dh), :], preferred_element_type=_F32)

        def static_head(h):
            head(h, lambda c: advance(n_pro + h * per_head + c))

        for h in range(_DEFERRED):
            static_head(h)

        z = vec_v[1] + jnp.dot(t_v[...], w4_v[...], preferred_element_type=_F32)
        vec_v[3] = z * jax.nn.sigmoid(z)

        def loop_head(h, carry):
            def advance_from(c):
                dh_, c_ = divmod(c + _AHEAD, per_head)
                start_el(head_el(h + dh_, c_))
            head(h, advance_from)
            return carry

        jax.lax.fori_loop(_DEFERRED, heads - 1, loop_head, 0)
        static_head(heads - 1)

        s = vec_v[2]
        for i in range(_DEFERRED):
            tail_copy(i).wait()
            s = s + jnp.dot(o_v[i], wo_v[i * dh:(i + 1) * dh, :], preferred_element_type=_F32)
        out = vec_v[0] + s * vec_v[3]
        out_ref[0] = out[0:1].astype(out_ref.dtype)

    dma = pltpu.SemaphoreType.DMA
    pl.run_scoped(body, dma((1,)), dma((n_pro,)), dma((n_pro,)), dma((per_head,)),
                  dma((per_head,)), dma((_WO_PIECES,)), dma((_DEFERRED,)))


@jax.jit
def pallas_recurrent_scan__sliding_block_cached__mixer_s_mlp__decode_kernel(
    A_x, A_k_cache, A_v_cache, A_wq, A_wo, B_x, B_w1, B_w2, B_w3, B_w4,
):
    b, sq, d = A_x.shape
    _, heads, seq, dh = A_k_cache.shape
    f = B_w3.shape[1]
    window = min(4096, max(256, seq // 4))
    assert b == 1 and sq == 1 and A_wq.shape[1] == heads * dh
    assert window % _CHUNK == 0 and f % 16 == 0
    assert _TAIL_GAP * _DEFERRED <= _AHEAD <= 2 * window // _KV_ROWS

    return pl.pallas_call(
        functools.partial(_kernel, heads=heads, window=window, seq=seq, dh=dh, d=d, f=f),
        in_specs=[pl.BlockSpec(memory_space=pl.ANY)] * 7,
        out_specs=pl.BlockSpec(memory_space=pltpu.VMEM),
        out_shape=jax.ShapeDtypeStruct((b, sq, d), A_x.dtype),
        scratch_shapes=[
            pltpu.VMEM((1, 1, d), _BF16),
            pltpu.VMEM((d, heads * dh), _BF16),
            pltpu.VMEM((2, window, dh), _BF16),
            pltpu.VMEM((2, window, dh), _BF16),
            pltpu.VMEM((heads * dh, d), _BF16),
            pltpu.VMEM((f, d), _BF16),
            pltpu.VMEM((f, d), _BF16),
            pltpu.VMEM((heads, _ROWS, dh), _BF16),
            pltpu.VMEM((_ROWS, f), _BF16),
            pltpu.VMEM((_DEFERRED, _ROWS, dh), _BF16),
            pltpu.VMEM((4, _ROWS, d), _F32),
        ],
        compiler_params=pltpu.CompilerParams(vmem_limit_bytes=32 * 1024 * 1024),
    )(A_x, A_wq, A_k_cache, A_v_cache, A_wo, B_w3.T, B_w4)
```

```python
import functools

import jax
import jax.numpy as jnp
import jax.experimental.pallas as pl
import jax.experimental.pallas.tpu as pltpu

_EPS = 1e-5
_F32 = jnp.float32
_BF16 = jnp.bfloat16
_NT = (((1,), (1,)), ((), ()))

_ROWS = 8
_KV_ROWS = 256
_KV_HI = 64
_WQ_ROWS = 8
_WQ_HI = 1024
_W_ROWS = 64
_W_HI = 16
_WO_PIECES = 8
_CHUNK = 1024
_AHEAD = 29
_DEFERRED = 3
_TAIL_GAP = 2
_VPU_ROWS = 64
_Q_STEPS = 4
_HI, _LO = 0, 1


def _layernorm(x):
    m = jnp.mean(x, axis=-1, keepdims=True)
    xc = x - m
    v = jnp.mean(xc * xc, axis=-1, keepdims=True)
    return xc / jnp.sqrt(v + _EPS)


def _kernel(x_hbm, wq_hbm, k_hbm, v_hbm, wo_hbm, w3t_hbm, w4_hbm, out_ref,
            x_v, wq_v, k_v, v_v, wo_v, w3t_v, w4_v, q_v, t_v, o_v, ocol_v, vec_v,
            *, heads, window, seq, dh, d, f):
    scale = dh ** -0.5
    n_pos = window // _KV_ROWS
    per_head = 2 * n_pos
    per_chunk = _CHUNK // _KV_ROWS
    chunks = window // _CHUNK
    piece = dh // _WO_PIECES
    every = per_head // _WO_PIECES
    first_key = seq - window
    w4_early = f - _DEFERRED * dh
    all_cols = slice(None)

    pro = [((wq_hbm, wq_v, pl.ds(r, _WQ_ROWS), pl.ds(0, _WQ_HI)),
            (wq_hbm, wq_v, pl.ds(r, _WQ_ROWS), pl.ds(_WQ_HI, heads * dh - _WQ_HI)))
           for r in range(0, d, _WQ_ROWS)]
    n_wq = len(pro)
    for src, dst, total in ((w3t_hbm, w3t_v, f), (w4_hbm, w4_v, w4_early)):
        for r in range(0, total, _W_ROWS):
            n = min(_W_ROWS, total - r)
            if n > _W_HI:
                pro.append(((src, dst, pl.ds(r, _W_HI), all_cols),
                            (src, dst, pl.ds(r + _W_HI, n - _W_HI), all_cols)))
            else:
                pro.append((None, (src, dst, pl.ds(r, n), all_cols)))
    n_pro = len(pro)
    n_el = n_pro + heads * per_head
    vpu_row0 = (_DEFERRED - 1) * dh
    tail = [(h * dh, dh) for h in range(_DEFERRED - 1)]
    tail += [(r, _VPU_ROWS) for r in range(vpu_row0, vpu_row0 + dh, _VPU_ROWS)]

    def body(sem_x, sem_pro_hi, sem_pro_lo, sem_hi, sem_lo, sem_piece, sem_tail):
        def block_copy(spec, sem):
            src, dst, rows, cols = spec
            return pltpu.make_async_copy(src.at[rows, cols], dst.at[rows, cols], sem)

        def pro_el(i):
            hi, lo = pro[i]
            his = [] if hi is None else [functools.partial(block_copy, hi, sem_pro_hi.at[i])]
            return his, functools.partial(block_copy, lo, sem_pro_lo.at[i])

        def head_el(h, c):
            static = isinstance(h, int)
            his = []
            if c % every == 0:
                w = c // every
                if static and h < _DEFERRED:
                    rows = pl.ds(w4_early + h * dh + w * piece, piece)
                    spec = (w4_hbm, w4_v, rows, all_cols)
                else:
                    r = h * dh + w * piece
                    r = r if static else pl.multiple_of(r, piece)
                    spec = (wo_hbm, wo_v, pl.ds(r, piece), all_cols)
                his.append(functools.partial(block_copy, spec, sem_piece.at[w]))
            src, dst, j = (k_hbm, k_v, c) if c < n_pos else (v_hbm, v_v, c - n_pos)

            def kv_copy(r, n, sem):
                return pltpu.make_async_copy(src.at[0, h, pl.ds(first_key + r, n), :],
                                             dst.at[h % 2, pl.ds(r, n), :], sem)

            his.append(functools.partial(kv_copy, j * _KV_ROWS, _KV_HI, sem_hi.at[c]))
            lo = functools.partial(kv_copy, j * _KV_ROWS + _KV_HI, _KV_ROWS - _KV_HI,
                                   sem_lo.at[c])
            return his, lo

        def element(i):
            return pro_el(i) if i < n_pro else head_el(*divmod(i - n_pro, per_head))

        def tail_copy(i):
            return block_copy((wo_hbm, wo_v, pl.ds(*tail[i]), all_cols), sem_tail.at[i])

        def start_el(el):
            for cp in el[0]:
                cp().start(priority=_HI)
            el[1]().start(priority=_LO)

        def wait_el(el):
            for cp in el[0]:
                cp().wait()
            el[1]().wait()

        def advance(i):
            j = i + _AHEAD
            if j < n_el:
                start_el(element(j))
            elif (j - n_el) % _TAIL_GAP == 0 and (j - n_el) // _TAIL_GAP < len(tail):
                tail_copy((j - n_el) // _TAIL_GAP).start(priority=_LO)

        x_copy = pltpu.make_async_copy(x_hbm, x_v, sem_x.at[0])
        x_copy.start()
        for i in range(_AHEAD):
            start_el(element(i))
        x_copy.wait()
        x = jnp.broadcast_to(x_v[0].astype(_F32), (_ROWS, d))
        xn = _layernorm(x)
        xn_b = xn.astype(_BF16)
        vec_v[0] = x
        vec_v[1] = xn
        vec_v[2] = jnp.zeros((_ROWS, d), _F32)

        q = None
        per_step = n_wq // _Q_STEPS
        for i in range(n_pro):
            wait_el(element(i))
            advance(i)
            if i < n_wq and (i + 1) % per_step == 0:
                r1 = (i + 1) * _WQ_ROWS
                r0 = r1 - per_step * _WQ_ROWS
                part = jnp.dot(xn_b[:, r0:r1], wq_v[r0:r1, :], preferred_element_type=_F32)
                q = part if q is None else q + part
                if i == n_wq - 1:
                    for h in range(heads):
                        q_v[h] = q[:, h * dh:(h + 1) * dh].astype(_BF16)
        hidden = jax.lax.dot_general(_layernorm(xn).astype(_BF16), w3t_v[...], _NT,
                                     preferred_element_type=_F32)
        t_v[...] = jax.nn.gelu(hidden, approximate=True).astype(_BF16)

        def head(h, advance_from):
            def arrive(first):
                for c in range(first, first + per_chunk):
                    wait_el(head_el(h, c))
                    advance_from(c)

            qh = q_v[h]
            scores = []
            for c in range(chunks):
                arrive(c * per_chunk)
                scores.append(jax.lax.dot_general(
                    qh, k_v[h % 2, pl.ds(c * _CHUNK, _CHUNK), :], _NT,
                    preferred_element_type=_F32))
            m = functools.reduce(
                jnp.maximum, [jnp.max(s, axis=-1, keepdims=True) for s in scores])
            p = [jnp.exp((s - m) * scale) for s in scores]
            l = functools.reduce(jnp.add, [jnp.sum(e, axis=-1, keepdims=True) for e in p])
            o = jnp.zeros((_ROWS, dh), _F32)
            for c in range(chunks):
                arrive(n_pos + c * per_chunk)
                o = o + jnp.dot(p[c].astype(_BF16),
                                v_v[h % 2, pl.ds(c * _CHUNK, _CHUNK), :],
                                preferred_element_type=_F32)
            o = (o / l).astype(_BF16)
            if isinstance(h, int) and h < _DEFERRED - 1:
                o_v[h] = o
            elif isinstance(h, int) and h == _DEFERRED - 1:
                ocol_v[...] = jnp.broadcast_to(o[0:1].astype(_F32), (dh, dh)).T
            else:
                r = h * dh if isinstance(h, int) else pl.multiple_of(h * dh, dh)
                vec_v[2] += jnp.dot(o, wo_v[pl.ds(r, dh), :], preferred_element_type=_F32)

        def static_head(h):
            head(h, lambda c: advance(n_pro + h * per_head + c))

        for h in range(_DEFERRED):
            static_head(h)

        z = vec_v[1] + jnp.dot(t_v[...], w4_v[...], preferred_element_type=_F32)
        vec_v[3] = z * jax.nn.sigmoid(z)

        def loop_head(h, carry):
            def advance_from(c):
                dh_, c_ = divmod(c + _AHEAD, per_head)
                start_el(head_el(h + dh_, c_))
            head(h, advance_from)
            return carry

        jax.lax.fori_loop(_DEFERRED, heads - 1, loop_head, 0)
        static_head(heads - 1)

        s = vec_v[2]
        partial = jnp.zeros((_ROWS, d), _F32)
        for i, (r0, n) in enumerate(tail):
            tail_copy(i).wait()
            if r0 < vpu_row0:
                s = s + jnp.dot(o_v[i], wo_v[r0:r0 + n, :], preferred_element_type=_F32)
            else:
                w = wo_v[r0:r0 + n, :].astype(_F32)
                for r in range(0, n, _ROWS):
                    col = ocol_v[pl.ds(r0 - vpu_row0 + r, _ROWS), :]
                    col = jnp.concatenate([col] * (d // dh), axis=1)
                    partial = partial + w[r:r + _ROWS, :] * col
        s = s[0:1] + jnp.sum(partial, axis=0, keepdims=True)
        out = vec_v[0][0:1] + s * vec_v[3][0:1]
        out_ref[0] = out.astype(out_ref.dtype)

    dma = pltpu.SemaphoreType.DMA
    pl.run_scoped(body, dma((1,)), dma((n_pro,)), dma((n_pro,)), dma((per_head,)),
                  dma((per_head,)), dma((_WO_PIECES,)), dma((len(tail),)))


@jax.jit
def pallas_recurrent_scan__sliding_block_cached__mixer_s_mlp__decode_kernel(
    A_x, A_k_cache, A_v_cache, A_wq, A_wo, B_x, B_w1, B_w2, B_w3, B_w4,
):
    b, sq, d = A_x.shape
    _, heads, seq, dh = A_k_cache.shape
    f = B_w3.shape[1]
    window = min(4096, max(256, seq // 4))
    assert b == 1 and sq == 1 and A_wq.shape[1] == heads * dh
    assert window % _CHUNK == 0 and f % 16 == 0
    assert _TAIL_GAP * (_DEFERRED - 1 + dh // _VPU_ROWS) <= _AHEAD <= 2 * window // _KV_ROWS
    assert d % dh == 0

    return pl.pallas_call(
        functools.partial(_kernel, heads=heads, window=window, seq=seq, dh=dh, d=d, f=f),
        in_specs=[pl.BlockSpec(memory_space=pl.ANY)] * 7,
        out_specs=pl.BlockSpec(memory_space=pltpu.VMEM),
        out_shape=jax.ShapeDtypeStruct((b, sq, d), A_x.dtype),
        scratch_shapes=[
            pltpu.VMEM((1, 1, d), _BF16),
            pltpu.VMEM((d, heads * dh), _BF16),
            pltpu.VMEM((2, window, dh), _BF16),
            pltpu.VMEM((2, window, dh), _BF16),
            pltpu.VMEM((heads * dh, d), _BF16),
            pltpu.VMEM((f, d), _BF16),
            pltpu.VMEM((f, d), _BF16),
            pltpu.VMEM((heads, _ROWS, dh), _BF16),
            pltpu.VMEM((_ROWS, f), _BF16),
            pltpu.VMEM((_DEFERRED - 1, _ROWS, dh), _BF16),
            pltpu.VMEM((dh, dh), _F32),
            pltpu.VMEM((4, _ROWS, d), _F32),
        ],
        compiler_params=pltpu.CompilerParams(vmem_limit_bytes=32 * 1024 * 1024),
    )(A_x, A_wq, A_k_cache, A_v_cache, A_wo, B_w3.T, B_w4)
```

```python
import functools

import jax
import jax.numpy as jnp
import jax.experimental.pallas as pl
import jax.experimental.pallas.tpu as pltpu

_EPS = 1e-5
_F32 = jnp.float32
_BF16 = jnp.bfloat16
_NT = (((1,), (1,)), ((), ()))

_ROWS = 8
_KV_ROWS = 1024
_KV_HI = 352
_WQ_ROWS = 8
_WQ_HI = 1024
_W_ROWS = 64
_W_HI = 16
_WO_PIECES = 8
_CHUNK = 1024
_AHEAD = 8
_PRO_AHEAD = 32
_DEFERRED = 3
_VPU_ROWS = 64
_Q_STEPS = 4
_HI, _LO = 0, 1


def _layernorm(x):
    m = jnp.mean(x, axis=-1, keepdims=True)
    xc = x - m
    v = jnp.mean(xc * xc, axis=-1, keepdims=True)
    return xc / jnp.sqrt(v + _EPS)


def _kernel(x_hbm, wq_hbm, k_hbm, v_hbm, wo_hbm, w3t_hbm, w4_hbm, out_ref,
            x_v, wq_v, k_v, v_v, wo_v, w3t_v, w4_v, q_v, t_v, o_v, ocol_v, vec_v,
            *, heads, window, seq, dh, d, f):
    scale = dh ** -0.5
    n_pos = window // _KV_ROWS
    per_head = 2 * n_pos
    per_chunk = _CHUNK // _KV_ROWS
    chunks = window // _CHUNK
    piece = dh // _WO_PIECES
    every = per_head // _WO_PIECES
    first_key = seq - window
    w4_early = f - _DEFERRED * dh
    all_cols = slice(None)

    pro = [((wq_hbm, wq_v, pl.ds(r, _WQ_ROWS), pl.ds(0, _WQ_HI)),
            (wq_hbm, wq_v, pl.ds(r, _WQ_ROWS), pl.ds(_WQ_HI, heads * dh - _WQ_HI)))
           for r in range(0, d, _WQ_ROWS)]
    n_wq = len(pro)
    for src, dst, total in ((w3t_hbm, w3t_v, f), (w4_hbm, w4_v, w4_early)):
        for r in range(0, total, _W_ROWS):
            n = min(_W_ROWS, total - r)
            if n > _W_HI:
                pro.append(((src, dst, pl.ds(r, _W_HI), all_cols),
                            (src, dst, pl.ds(r + _W_HI, n - _W_HI), all_cols)))
            else:
                pro.append((None, (src, dst, pl.ds(r, n), all_cols)))
    n_pro = len(pro)
    n_el = n_pro + heads * per_head
    vpu_row0 = (_DEFERRED - 1) * dh
    tail = [(h * dh, dh) for h in range(_DEFERRED - 1)]
    tail += [(r, _VPU_ROWS) for r in range(vpu_row0, vpu_row0 + dh, _VPU_ROWS)]

    def body(sem_x, sem_pro_hi, sem_pro_lo, sem_hi, sem_lo, sem_piece, sem_tail):
        def block_copy(spec, sem):
            src, dst, rows, cols = spec
            return pltpu.make_async_copy(src.at[rows, cols], dst.at[rows, cols], sem)

        def pro_el(i):
            hi, lo = pro[i]
            his = [] if hi is None else [functools.partial(block_copy, hi, sem_pro_hi.at[i])]
            return his, functools.partial(block_copy, lo, sem_pro_lo.at[i])

        def head_el(h, c):
            static = isinstance(h, int)
            his = []
            if c % every == 0:
                w = c // every
                if static and h < _DEFERRED:
                    rows = pl.ds(w4_early + h * dh + w * piece, piece)
                    spec = (w4_hbm, w4_v, rows, all_cols)
                else:
                    r = h * dh + w * piece
                    r = r if static else pl.multiple_of(r, piece)
                    spec = (wo_hbm, wo_v, pl.ds(r, piece), all_cols)
                his.append(functools.partial(block_copy, spec, sem_piece.at[w]))
            src, dst, j = (k_hbm, k_v, c) if c < n_pos else (v_hbm, v_v, c - n_pos)

            def kv_copy(r, n, sem):
                return pltpu.make_async_copy(src.at[0, h, pl.ds(first_key + r, n), :],
                                             dst.at[h % 2, pl.ds(r, n), :], sem)

            his.append(functools.partial(kv_copy, j * _KV_ROWS, _KV_HI, sem_hi.at[c]))
            lo = functools.partial(kv_copy, j * _KV_ROWS + _KV_HI, _KV_ROWS - _KV_HI,
                                   sem_lo.at[c])
            return his, lo

        def element(i):
            return pro_el(i) if i < n_pro else head_el(*divmod(i - n_pro, per_head))

        def tail_copy(i):
            return block_copy((wo_hbm, wo_v, pl.ds(*tail[i]), all_cols), sem_tail.at[i])

        def start_el(el):
            for cp in el[0]:
                cp().start(priority=_HI)
            el[1]().start(priority=_LO)

        def wait_el(el):
            for cp in el[0]:
                cp().wait()
            el[1]().wait()

        def advance_pro(i):
            j = i + _PRO_AHEAD
            if j < n_pro:
                start_el(element(j))
            else:
                for k in range((j - n_pro) * _AHEAD // _PRO_AHEAD,
                               (j - n_pro + 1) * _AHEAD // _PRO_AHEAD):
                    start_el(element(n_pro + k))

        def advance(i):
            j = i + _AHEAD
            if j < n_el:
                start_el(element(j))
            elif j - n_el < len(tail):
                tail_copy(j - n_el).start(priority=_LO)

        x_copy = pltpu.make_async_copy(x_hbm, x_v, sem_x.at[0])
        x_copy.start()
        for i in range(_PRO_AHEAD):
            start_el(element(i))
        x_copy.wait()
        x = jnp.broadcast_to(x_v[0].astype(_F32), (_ROWS, d))
        xn = _layernorm(x)
        xn_b = xn.astype(_BF16)
        vec_v[0] = x
        vec_v[1] = xn
        vec_v[2] = jnp.zeros((_ROWS, d), _F32)

        q = None
        per_step = n_wq // _Q_STEPS
        for i in range(n_pro):
            wait_el(element(i))
            advance_pro(i)
            if i < n_wq and (i + 1) % per_step == 0:
                r1 = (i + 1) * _WQ_ROWS
                r0 = r1 - per_step * _WQ_ROWS
                part = jnp.dot(xn_b[:, r0:r1], wq_v[r0:r1, :], preferred_element_type=_F32)
                q = part if q is None else q + part
                if i == n_wq - 1:
                    for h in range(heads):
                        q_v[h] = q[:, h * dh:(h + 1) * dh].astype(_BF16)
        hidden = jax.lax.dot_general(_layernorm(xn).astype(_BF16), w3t_v[...], _NT,
                                     preferred_element_type=_F32)
        t_v[...] = jax.nn.gelu(hidden, approximate=True).astype(_BF16)

        def head(h, advance_from):
            def arrive(first):
                for c in range(first, first + per_chunk):
                    wait_el(head_el(h, c))
                    advance_from(c)

            qh = q_v[h]
            scores = []
            for c in range(chunks):
                arrive(c * per_chunk)
                scores.append(jax.lax.dot_general(
                    qh, k_v[h % 2, pl.ds(c * _CHUNK, _CHUNK), :], _NT,
                    preferred_element_type=_F32))
            m = functools.reduce(
                jnp.maximum, [jnp.max(s, axis=-1, keepdims=True) for s in scores])
            p = [jnp.exp((s - m) * scale) for s in scores]
            l = functools.reduce(jnp.add, [jnp.sum(e, axis=-1, keepdims=True) for e in p])
            o = jnp.zeros((_ROWS, dh), _F32)
            for c in range(chunks):
                arrive(n_pos + c * per_chunk)
                o = o + jnp.dot(p[c].astype(_BF16),
                                v_v[h % 2, pl.ds(c * _CHUNK, _CHUNK), :],
                                preferred_element_type=_F32)
            o = (o / l).astype(_BF16)
            if isinstance(h, int) and h < _DEFERRED - 1:
                o_v[h] = o
            elif isinstance(h, int) and h == _DEFERRED - 1:
                ocol_v[...] = jnp.broadcast_to(o[0:1].astype(_F32), (dh, dh)).T
            else:
                r = h * dh if isinstance(h, int) else pl.multiple_of(h * dh, dh)
                vec_v[2] += jnp.dot(o, wo_v[pl.ds(r, dh), :], preferred_element_type=_F32)

        def static_head(h):
            head(h, lambda c: advance(n_pro + h * per_head + c))

        for h in range(_DEFERRED):
            static_head(h)

        z = vec_v[1] + jnp.dot(t_v[...], w4_v[...], preferred_element_type=_F32)
        vec_v[3] = z * jax.nn.sigmoid(z)

        def loop_head(h, carry):
            def advance_from(c):
                dh_, c_ = divmod(c + _AHEAD, per_head)
                start_el(head_el(h + dh_, c_))
            head(h, advance_from)
            return carry

        jax.lax.fori_loop(_DEFERRED, heads - 1, loop_head, 0)
        static_head(heads - 1)

        s = vec_v[2]
        partial = jnp.zeros((_ROWS, d), _F32)
        for i, (r0, n) in enumerate(tail):
            tail_copy(i).wait()
            if r0 < vpu_row0:
                s = s + jnp.dot(o_v[i], wo_v[r0:r0 + n, :], preferred_element_type=_F32)
            else:
                w = wo_v[r0:r0 + n, :].astype(_F32)
                for r in range(0, n, _ROWS):
                    col = ocol_v[pl.ds(r0 - vpu_row0 + r, _ROWS), :]
                    col = jnp.concatenate([col] * (d // dh), axis=1)
                    partial = partial + w[r:r + _ROWS, :] * col
        s = s[0:1] + jnp.sum(partial, axis=0, keepdims=True)
        out = vec_v[0][0:1] + s * vec_v[3][0:1]
        out_ref[0] = out.astype(out_ref.dtype)

    dma = pltpu.SemaphoreType.DMA
    pl.run_scoped(body, dma((1,)), dma((n_pro,)), dma((n_pro,)), dma((per_head,)),
                  dma((per_head,)), dma((_WO_PIECES,)), dma((len(tail),)))


@jax.jit
def pallas_recurrent_scan__sliding_block_cached__mixer_s_mlp__decode_kernel(
    A_x, A_k_cache, A_v_cache, A_wq, A_wo, B_x, B_w1, B_w2, B_w3, B_w4,
):
    b, sq, d = A_x.shape
    _, heads, seq, dh = A_k_cache.shape
    f = B_w3.shape[1]
    window = min(4096, max(256, seq // 4))
    assert b == 1 and sq == 1 and A_wq.shape[1] == heads * dh
    assert window % _CHUNK == 0 and f % 16 == 0
    assert _DEFERRED - 1 + dh // _VPU_ROWS <= _AHEAD <= 2 * window // _KV_ROWS
    assert d % dh == 0

    return pl.pallas_call(
        functools.partial(_kernel, heads=heads, window=window, seq=seq, dh=dh, d=d, f=f),
        in_specs=[pl.BlockSpec(memory_space=pl.ANY)] * 7,
        out_specs=pl.BlockSpec(memory_space=pltpu.VMEM),
        out_shape=jax.ShapeDtypeStruct((b, sq, d), A_x.dtype),
        scratch_shapes=[
            pltpu.VMEM((1, 1, d), _BF16),
            pltpu.VMEM((d, heads * dh), _BF16),
            pltpu.VMEM((2, window, dh), _BF16),
            pltpu.VMEM((2, window, dh), _BF16),
            pltpu.VMEM((heads * dh, d), _BF16),
            pltpu.VMEM((f, d), _BF16),
            pltpu.VMEM((f, d), _BF16),
            pltpu.VMEM((heads, _ROWS, dh), _BF16),
            pltpu.VMEM((_ROWS, f), _BF16),
            pltpu.VMEM((_DEFERRED - 1, _ROWS, dh), _BF16),
            pltpu.VMEM((dh, dh), _F32),
            pltpu.VMEM((4, _ROWS, d), _F32),
        ],
        compiler_params=pltpu.CompilerParams(vmem_limit_bytes=32 * 1024 * 1024),
    )(A_x, A_wq, A_k_cache, A_v_cache, A_wo, B_w3.T, B_w4)
```

```python
import functools

import jax
import jax.numpy as jnp
import jax.experimental.pallas as pl
import jax.experimental.pallas.tpu as pltpu

_EPS = 1e-5
_F32 = jnp.float32
_BF16 = jnp.bfloat16
_NT = (((1,), (1,)), ((), ()))

_ROWS = 8
_KV_ROWS = 256
_KV_HI = 88
_WQ_ROWS = 8
_WQ_HI = 1024
_W_ROWS = 64
_W_HI = 16
_WO_PIECES = 8
_CHUNK = 1024
_AHEAD = 29
_DEFERRED = 3
_VPU_ROWS = 64
_Q_STEPS = 4
_HI, _LO = 0, 1


def _layernorm(x):
    m = jnp.mean(x, axis=-1, keepdims=True)
    xc = x - m
    v = jnp.mean(xc * xc, axis=-1, keepdims=True)
    return xc / jnp.sqrt(v + _EPS)


def _kernel(x_hbm, wq_hbm, k_hbm, v_hbm, wo_hbm, w3t_hbm, w4_hbm, out_ref,
            x_v, wq_v, k_v, v_v, wo_v, w3t_v, w4_v, q_v, t_v, o_v, ocol_v, vec_v,
            *, heads, window, seq, dh, d, f):
    scale = dh ** -0.5
    n_pos = window // _KV_ROWS
    per_head = 2 * n_pos
    per_chunk = _CHUNK // _KV_ROWS
    chunks = window // _CHUNK
    piece = dh // _WO_PIECES
    every = per_head // _WO_PIECES
    first_key = seq - window
    w4_early = f - _DEFERRED * dh
    all_cols = slice(None)

    pro = [((wq_hbm, wq_v, pl.ds(r, _WQ_ROWS), pl.ds(0, _WQ_HI)),
            (wq_hbm, wq_v, pl.ds(r, _WQ_ROWS), pl.ds(_WQ_HI, heads * dh - _WQ_HI)))
           for r in range(0, d, _WQ_ROWS)]
    n_wq = len(pro)
    for src, dst, total in ((w3t_hbm, w3t_v, f), (w4_hbm, w4_v, w4_early)):
        for r in range(0, total, _W_ROWS):
            n = min(_W_ROWS, total - r)
            if n > _W_HI:
                pro.append(((src, dst, pl.ds(r, _W_HI), all_cols),
                            (src, dst, pl.ds(r + _W_HI, n - _W_HI), all_cols)))
            else:
                pro.append((None, (src, dst, pl.ds(r, n), all_cols)))
    n_pro = len(pro)
    n_el = n_pro + heads * per_head
    vpu_row0 = (_DEFERRED - 1) * dh
    tail = [(h * dh, dh) for h in range(_DEFERRED - 1)]
    tail += [(r, _VPU_ROWS) for r in range(vpu_row0, vpu_row0 + dh, _VPU_ROWS)]

    def body(sem_x, sem_pro_hi, sem_pro_lo, sem_hi, sem_lo, sem_piece, sem_tail):
        def block_copy(spec, sem):
            src, dst, rows, cols = spec
            return pltpu.make_async_copy(src.at[rows, cols], dst.at[rows, cols], sem)

        def pro_el(i):
            hi, lo = pro[i]
            his = [] if hi is None else [functools.partial(block_copy, hi, sem_pro_hi.at[i])]
            return his, functools.partial(block_copy, lo, sem_pro_lo.at[i])

        def head_el(h, c):
            static = isinstance(h, int)
            his = []
            if c % every == 0:
                w = c // every
                if static and h < _DEFERRED:
                    rows = pl.ds(w4_early + h * dh + w * piece, piece)
                    spec = (w4_hbm, w4_v, rows, all_cols)
                else:
                    r = h * dh + w * piece
                    r = r if static else pl.multiple_of(r, piece)
                    spec = (wo_hbm, wo_v, pl.ds(r, piece), all_cols)
                his.append(functools.partial(block_copy, spec, sem_piece.at[w]))
            src, dst, j = (k_hbm, k_v, c) if c < n_pos else (v_hbm, v_v, c - n_pos)

            def kv_copy(key, row, n, sem):
                return pltpu.make_async_copy(src.at[0, h, pl.ds(first_key + key, n), :],
                                             dst.at[h % 2, pl.ds(row, n), :], sem)

            n_lo = _KV_ROWS - _KV_HI
            his.append(functools.partial(kv_copy, j * _KV_HI, j * _KV_ROWS, _KV_HI,
                                         sem_hi.at[c]))
            lo = functools.partial(kv_copy, n_pos * _KV_HI + j * n_lo, j * _KV_ROWS + _KV_HI,
                                   n_lo, sem_lo.at[c])
            return his, lo

        def element(i):
            return pro_el(i) if i < n_pro else head_el(*divmod(i - n_pro, per_head))

        def tail_copy(i):
            return block_copy((wo_hbm, wo_v, pl.ds(*tail[i]), all_cols), sem_tail.at[i])

        def start_el(el):
            for cp in el[0]:
                cp().start(priority=_HI)
            el[1]().start(priority=_LO)

        def wait_el(el):
            for cp in el[0]:
                cp().wait()
            el[1]().wait()

        def advance(i):
            j = i + _AHEAD
            if j < n_el:
                start_el(element(j))
            elif j - n_el < len(tail):
                tail_copy(j - n_el).start(priority=_LO)

        x_copy = pltpu.make_async_copy(x_hbm, x_v, sem_x.at[0])
        x_copy.start()
        for i in range(_AHEAD):
            start_el(element(i))
        x_copy.wait()
        x = jnp.broadcast_to(x_v[0].astype(_F32), (_ROWS, d))
        xn = _layernorm(x)
        xn_b = xn.astype(_BF16)
        vec_v[0] = x
        vec_v[1] = xn
        vec_v[2] = jnp.zeros((_ROWS, d), _F32)

        q = None
        per_step = n_wq // _Q_STEPS
        for i in range(n_pro):
            wait_el(element(i))
            advance(i)
            if i < n_wq and (i + 1) % per_step == 0:
                r1 = (i + 1) * _WQ_ROWS
                r0 = r1 - per_step * _WQ_ROWS
                part = jnp.dot(xn_b[:, r0:r1], wq_v[r0:r1, :], preferred_element_type=_F32)
                q = part if q is None else q + part
                if i == n_wq - 1:
                    for h in range(heads):
                        q_v[h] = q[:, h * dh:(h + 1) * dh].astype(_BF16)
        hidden = jax.lax.dot_general(_layernorm(xn).astype(_BF16), w3t_v[...], _NT,
                                     preferred_element_type=_F32)
        t_v[...] = jax.nn.gelu(hidden, approximate=True).astype(_BF16)

        def head(h, advance_from):
            def arrive(first):
                for c in range(first, first + per_chunk):
                    wait_el(head_el(h, c))
                    advance_from(c)

            qh = q_v[h]
            scores = []
            for c in range(chunks):
                arrive(c * per_chunk)
                scores.append(jax.lax.dot_general(
                    qh, k_v[h % 2, pl.ds(c * _CHUNK, _CHUNK), :], _NT,
                    preferred_element_type=_F32))
            m = functools.reduce(
                jnp.maximum, [jnp.max(s, axis=-1, keepdims=True) for s in scores])
            p = [jnp.exp((s - m) * scale) for s in scores]
            l = functools.reduce(jnp.add, [jnp.sum(e, axis=-1, keepdims=True) for e in p])
            o = jnp.zeros((_ROWS, dh), _F32)
            for c in range(chunks):
                arrive(n_pos + c * per_chunk)
                o = o + jnp.dot(p[c].astype(_BF16),
                                v_v[h % 2, pl.ds(c * _CHUNK, _CHUNK), :],
                                preferred_element_type=_F32)
            o = (o / l).astype(_BF16)
            if isinstance(h, int) and h < _DEFERRED - 1:
                o_v[h] = o
            elif isinstance(h, int) and h == _DEFERRED - 1:
                ocol_v[...] = jnp.broadcast_to(o[0:1].astype(_F32), (dh, dh)).T
            else:
                r = h * dh if isinstance(h, int) else pl.multiple_of(h * dh, dh)
                vec_v[2] += jnp.dot(o, wo_v[pl.ds(r, dh), :], preferred_element_type=_F32)

        def static_head(h):
            head(h, lambda c: advance(n_pro + h * per_head + c))

        for h in range(_DEFERRED):
            static_head(h)

        z = vec_v[1] + jnp.dot(t_v[...], w4_v[...], preferred_element_type=_F32)
        vec_v[3] = z * jax.nn.sigmoid(z)

        def loop_head(h, carry):
            def advance_from(c):
                dh_, c_ = divmod(c + _AHEAD, per_head)
                start_el(head_el(h + dh_, c_))
            head(h, advance_from)
            return carry

        jax.lax.fori_loop(_DEFERRED, heads - 1, loop_head, 0)
        static_head(heads - 1)

        s = vec_v[2]
        partial = jnp.zeros((_ROWS, d), _F32)
        for i, (r0, n) in enumerate(tail):
            tail_copy(i).wait()
            if r0 < vpu_row0:
                s = s + jnp.dot(o_v[i], wo_v[r0:r0 + n, :], preferred_element_type=_F32)
            else:
                w = wo_v[r0:r0 + n, :].astype(_F32)
                for r in range(0, n, _ROWS):
                    col = ocol_v[pl.ds(r0 - vpu_row0 + r, _ROWS), :]
                    col = jnp.concatenate([col] * (d // dh), axis=1)
                    partial = partial + w[r:r + _ROWS, :] * col
        s = s[0:1] + jnp.sum(partial, axis=0, keepdims=True)
        out = vec_v[0][0:1] + s * vec_v[3][0:1]
        out_ref[0] = out.astype(out_ref.dtype)

    dma = pltpu.SemaphoreType.DMA
    pl.run_scoped(body, dma((1,)), dma((n_pro,)), dma((n_pro,)), dma((per_head,)),
                  dma((per_head,)), dma((_WO_PIECES,)), dma((len(tail),)))


@jax.jit
def pallas_recurrent_scan__sliding_block_cached__mixer_s_mlp__decode_kernel(
    A_x, A_k_cache, A_v_cache, A_wq, A_wo, B_x, B_w1, B_w2, B_w3, B_w4,
):
    b, sq, d = A_x.shape
    _, heads, seq, dh = A_k_cache.shape
    f = B_w3.shape[1]
    window = min(4096, max(256, seq // 4))
    assert b == 1 and sq == 1 and A_wq.shape[1] == heads * dh
    assert window % _CHUNK == 0 and f % 16 == 0
    assert _DEFERRED - 1 + dh // _VPU_ROWS <= _AHEAD <= 2 * window // _KV_ROWS
    assert d % dh == 0

    return pl.pallas_call(
        functools.partial(_kernel, heads=heads, window=window, seq=seq, dh=dh, d=d, f=f),
        in_specs=[pl.BlockSpec(memory_space=pl.ANY)] * 7,
        out_specs=pl.BlockSpec(memory_space=pltpu.VMEM),
        out_shape=jax.ShapeDtypeStruct((b, sq, d), A_x.dtype),
        scratch_shapes=[
            pltpu.VMEM((1, 1, d), _BF16),
            pltpu.VMEM((d, heads * dh), _BF16),
            pltpu.VMEM((2, window, dh), _BF16),
            pltpu.VMEM((2, window, dh), _BF16),
            pltpu.VMEM((heads * dh, d), _BF16),
            pltpu.VMEM((f, d), _BF16),
            pltpu.VMEM((f, d), _BF16),
            pltpu.VMEM((heads, _ROWS, dh), _BF16),
            pltpu.VMEM((_ROWS, f), _BF16),
            pltpu.VMEM((_DEFERRED - 1, _ROWS, dh), _BF16),
            pltpu.VMEM((dh, dh), _F32),
            pltpu.VMEM((4, _ROWS, d), _F32),
        ],
        compiler_params=pltpu.CompilerParams(vmem_limit_bytes=32 * 1024 * 1024),
    )(A_x, A_wq, A_k_cache, A_v_cache, A_wo, B_w3.T, B_w4)
```

```python
import functools

import jax
import jax.numpy as jnp
import jax.experimental.pallas as pl
import jax.experimental.pallas.tpu as pltpu

_EPS = 1e-5
_F32 = jnp.float32
_BF16 = jnp.bfloat16
_NT = (((1,), (1,)), ((), ()))

_ROWS = 8
_KV_ROWS = 256
_KV_HI = 80
_SUB = 2
_WQ_ROWS = 8
_WQ_HI = 1024
_W_ROWS = 64
_W_HI = 16
_WO_PIECES = 8
_CHUNK = 1024
_AHEAD = 29
_DEFERRED = 3
_VPU_ROWS = 64
_Q_STEPS = 4
_HI, _LO = 0, 1


def _layernorm(x):
    m = jnp.mean(x, axis=-1, keepdims=True)
    xc = x - m
    v = jnp.mean(xc * xc, axis=-1, keepdims=True)
    return xc / jnp.sqrt(v + _EPS)


def _kernel(x_hbm, wq_hbm, k_hbm, v_hbm, wo_hbm, w3t_hbm, w4_hbm, out_ref,
            x_v, wq_v, k_v, v_v, wo_v, w3t_v, w4_v, q_v, t_v, o_v, ocol_v, vec_v,
            *, heads, window, seq, dh, d, f):
    scale = dh ** -0.5
    n_pos = window // _KV_ROWS
    per_head = 2 * n_pos
    per_chunk = _CHUNK // _KV_ROWS
    chunks = window // _CHUNK
    piece = dh // _WO_PIECES
    every = per_head // _WO_PIECES
    sub_rows = window // _SUB
    first_sub = seq // sub_rows - _SUB
    w4_early = f - _DEFERRED * dh
    all_cols = slice(None)

    pro = [((wq_hbm, wq_v, pl.ds(r, _WQ_ROWS), pl.ds(0, _WQ_HI)),
            (wq_hbm, wq_v, pl.ds(r, _WQ_ROWS), pl.ds(_WQ_HI, heads * dh - _WQ_HI)))
           for r in range(0, d, _WQ_ROWS)]
    n_wq = len(pro)
    for src, dst, total in ((w3t_hbm, w3t_v, f), (w4_hbm, w4_v, w4_early)):
        for r in range(0, total, _W_ROWS):
            n = min(_W_ROWS, total - r)
            if n > _W_HI:
                pro.append(((src, dst, pl.ds(r, _W_HI), all_cols),
                            (src, dst, pl.ds(r + _W_HI, n - _W_HI), all_cols)))
            else:
                pro.append((None, (src, dst, pl.ds(r, n), all_cols)))
    n_pro = len(pro)
    n_el = n_pro + heads * per_head
    vpu_row0 = (_DEFERRED - 1) * dh
    tail = [(h * dh, dh) for h in range(_DEFERRED - 1)]
    tail += [(r, _VPU_ROWS) for r in range(vpu_row0, vpu_row0 + dh, _VPU_ROWS)]

    def body(sem_x, sem_pro_hi, sem_pro_lo, sem_hi, sem_lo, sem_piece, sem_tail):
        def block_copy(spec, sem):
            src, dst, rows, cols = spec
            return pltpu.make_async_copy(src.at[rows, cols], dst.at[rows, cols], sem)

        def pro_el(i):
            hi, lo = pro[i]
            his = [] if hi is None else [functools.partial(block_copy, hi, sem_pro_hi.at[i])]
            return his, functools.partial(block_copy, lo, sem_pro_lo.at[i])

        def head_el(h, c):
            static = isinstance(h, int)
            his = []
            if c % every == 0:
                w = c // every
                if static and h < _DEFERRED:
                    rows = pl.ds(w4_early + h * dh + w * piece, piece)
                    spec = (w4_hbm, w4_v, rows, all_cols)
                else:
                    r = h * dh + w * piece
                    r = r if static else pl.multiple_of(r, piece)
                    spec = (wo_hbm, wo_v, pl.ds(r, piece), all_cols)
                his.append(functools.partial(block_copy, spec, sem_piece.at[w]))
            src, dst, j = (k_hbm, k_v, c) if c < n_pos else (v_hbm, v_v, c - n_pos)

            def kv_copy(key, row, n, sem):
                return pltpu.make_async_copy(
                    src.at[0, h, pl.ds(first_sub, _SUB), pl.ds(key, n), :],
                    dst.at[h % 2, :, pl.ds(row, n), :], sem)

            n_hi, n_lo = _KV_HI // _SUB, (_KV_ROWS - _KV_HI) // _SUB
            row = j * (n_hi + n_lo)
            his.append(functools.partial(kv_copy, j * n_hi, row, n_hi, sem_hi.at[c]))
            lo = functools.partial(kv_copy, n_pos * n_hi + j * n_lo, row + n_hi, n_lo,
                                   sem_lo.at[c])
            return his, lo

        def element(i):
            return pro_el(i) if i < n_pro else head_el(*divmod(i - n_pro, per_head))

        def tail_copy(i):
            return block_copy((wo_hbm, wo_v, pl.ds(*tail[i]), all_cols), sem_tail.at[i])

        def start_el(el):
            for cp in el[0]:
                cp().start(priority=_HI)
            el[1]().start(priority=_LO)

        def wait_el(el):
            for cp in el[0]:
                cp().wait()
            el[1]().wait()

        def advance(i):
            j = i + _AHEAD
            if j < n_el:
                start_el(element(j))
            elif j - n_el < len(tail):
                tail_copy(j - n_el).start(priority=_LO)

        x_copy = pltpu.make_async_copy(x_hbm, x_v, sem_x.at[0])
        x_copy.start()
        for i in range(_AHEAD):
            start_el(element(i))
        x_copy.wait()
        x = jnp.broadcast_to(x_v[0].astype(_F32), (_ROWS, d))
        xn = _layernorm(x)
        xn_b = xn.astype(_BF16)
        vec_v[0] = x
        vec_v[1] = xn
        vec_v[2] = jnp.zeros((_ROWS, d), _F32)

        q = None
        per_step = n_wq // _Q_STEPS
        for i in range(n_pro):
            wait_el(element(i))
            advance(i)
            if i < n_wq and (i + 1) % per_step == 0:
                r1 = (i + 1) * _WQ_ROWS
                r0 = r1 - per_step * _WQ_ROWS
                part = jnp.dot(xn_b[:, r0:r1], wq_v[r0:r1, :], preferred_element_type=_F32)
                q = part if q is None else q + part
                if i == n_wq - 1:
                    for h in range(heads):
                        q_v[h] = q[:, h * dh:(h + 1) * dh].astype(_BF16)
        hidden = jax.lax.dot_general(_layernorm(xn).astype(_BF16), w3t_v[...], _NT,
                                     preferred_element_type=_F32)
        t_v[...] = jax.nn.gelu(hidden, approximate=True).astype(_BF16)

        def head(h, advance_from):
            def arrive(first):
                for c in range(first, first + per_chunk):
                    wait_el(head_el(h, c))
                    advance_from(c)

            def chunk(ref, c):
                n = _CHUNK // _SUB
                return ref[h % 2, :, pl.ds(c * n, n), :].reshape(_CHUNK, dh)

            qh = q_v[h]
            scores = []
            for c in range(chunks):
                arrive(c * per_chunk)
                scores.append(jax.lax.dot_general(qh, chunk(k_v, c), _NT,
                                                  preferred_element_type=_F32))
            m = functools.reduce(
                jnp.maximum, [jnp.max(s, axis=-1, keepdims=True) for s in scores])
            p = [jnp.exp((s - m) * scale) for s in scores]
            l = functools.reduce(jnp.add, [jnp.sum(e, axis=-1, keepdims=True) for e in p])
            o = jnp.zeros((_ROWS, dh), _F32)
            for c in range(chunks):
                arrive(n_pos + c * per_chunk)
                o = o + jnp.dot(p[c].astype(_BF16), chunk(v_v, c),
                                preferred_element_type=_F32)
            o = (o / l).astype(_BF16)
            if isinstance(h, int) and h < _DEFERRED - 1:
                o_v[h] = o
            elif isinstance(h, int) and h == _DEFERRED - 1:
                ocol_v[...] = jnp.broadcast_to(o[0:1].astype(_F32), (dh, dh)).T
            else:
                r = h * dh if isinstance(h, int) else pl.multiple_of(h * dh, dh)
                vec_v[2] += jnp.dot(o, wo_v[pl.ds(r, dh), :], preferred_element_type=_F32)

        def static_head(h):
            head(h, lambda c: advance(n_pro + h * per_head + c))

        for h in range(_DEFERRED):
            static_head(h)

        z = vec_v[1] + jnp.dot(t_v[...], w4_v[...], preferred_element_type=_F32)
        vec_v[3] = z * jax.nn.sigmoid(z)

        def loop_head(h, carry):
            def advance_from(c):
                dh_, c_ = divmod(c + _AHEAD, per_head)
                start_el(head_el(h + dh_, c_))
            head(h, advance_from)
            return carry

        jax.lax.fori_loop(_DEFERRED, heads - 1, loop_head, 0)
        static_head(heads - 1)

        s = vec_v[2]
        partial = jnp.zeros((_ROWS, d), _F32)
        for i, (r0, n) in enumerate(tail):
            tail_copy(i).wait()
            if r0 < vpu_row0:
                s = s + jnp.dot(o_v[i], wo_v[r0:r0 + n, :], preferred_element_type=_F32)
            else:
                w = wo_v[r0:r0 + n, :].astype(_F32)
                for r in range(0, n, _ROWS):
                    col = ocol_v[pl.ds(r0 - vpu_row0 + r, _ROWS), :]
                    col = jnp.concatenate([col] * (d // dh), axis=1)
                    partial = partial + w[r:r + _ROWS, :] * col
        s = s[0:1] + jnp.sum(partial, axis=0, keepdims=True)
        out = vec_v[0][0:1] + s * vec_v[3][0:1]
        out_ref[0] = out.astype(out_ref.dtype)

    dma = pltpu.SemaphoreType.DMA
    pl.run_scoped(body, dma((1,)), dma((n_pro,)), dma((n_pro,)), dma((per_head,)),
                  dma((per_head,)), dma((_WO_PIECES,)), dma((len(tail),)))


@jax.jit
def pallas_recurrent_scan__sliding_block_cached__mixer_s_mlp__decode_kernel(
    A_x, A_k_cache, A_v_cache, A_wq, A_wo, B_x, B_w1, B_w2, B_w3, B_w4,
):
    b, sq, d = A_x.shape
    _, heads, seq, dh = A_k_cache.shape
    f = B_w3.shape[1]
    window = min(4096, max(256, seq // 4))
    assert b == 1 and sq == 1 and A_wq.shape[1] == heads * dh
    assert window % _CHUNK == 0 and seq % (window // _SUB) == 0 and f % 16 == 0
    assert _DEFERRED - 1 + dh // _VPU_ROWS <= _AHEAD <= 2 * window // _KV_ROWS
    assert d % dh == 0

    def by_sub_block(cache):
        return cache.reshape(b, heads, seq * _SUB // window, window // _SUB, dh)

    return pl.pallas_call(
        functools.partial(_kernel, heads=heads, window=window, seq=seq, dh=dh, d=d, f=f),
        in_specs=[pl.BlockSpec(memory_space=pl.ANY)] * 7,
        out_specs=pl.BlockSpec(memory_space=pltpu.VMEM),
        out_shape=jax.ShapeDtypeStruct((b, sq, d), A_x.dtype),
        scratch_shapes=[
            pltpu.VMEM((1, 1, d), _BF16),
            pltpu.VMEM((d, heads * dh), _BF16),
            pltpu.VMEM((2, _SUB, window // _SUB, dh), _BF16),
            pltpu.VMEM((2, _SUB, window // _SUB, dh), _BF16),
            pltpu.VMEM((heads * dh, d), _BF16),
            pltpu.VMEM((f, d), _BF16),
            pltpu.VMEM((f, d), _BF16),
            pltpu.VMEM((heads, _ROWS, dh), _BF16),
            pltpu.VMEM((_ROWS, f), _BF16),
            pltpu.VMEM((_DEFERRED - 1, _ROWS, dh), _BF16),
            pltpu.VMEM((dh, dh), _F32),
            pltpu.VMEM((4, _ROWS, d), _F32),
        ],
        compiler_params=pltpu.CompilerParams(vmem_limit_bytes=32 * 1024 * 1024),
    )(A_x, A_wq, by_sub_block(A_k_cache), by_sub_block(A_v_cache), A_wo, B_w3.T, B_w4)
```

```python
import functools

import jax
import jax.numpy as jnp
import jax.experimental.pallas as pl
import jax.experimental.pallas.tpu as pltpu

_EPS = 1e-5
_F32 = jnp.float32
_BF16 = jnp.bfloat16
_NT = (((1,), (1,)), ((), ()))

_ROWS = 8
_GROUP = 4
_SEG = 16
_BLOCK = 8
_LO_AHEAD = 8
_HI_AHEAD = 4
_WQ_ROWS = 8
_WQ_HI = 1024
_W_ROWS = 64
_W_HI = 16
_PRO_AHEAD = 32
_Q_STEPS = 4
_VPU_ROWS = 64
_HI, _LO = 0, 1


def _layernorm(x):
    m = jnp.mean(x, axis=-1, keepdims=True)
    xc = x - m
    v = jnp.mean(xc * xc, axis=-1, keepdims=True)
    return xc / jnp.sqrt(v + _EPS)


def _aligned(x, m):
    return x if isinstance(x, int) else pl.multiple_of(x, m)


def _mod_pow2(x, m):
    assert m & (m - 1) == 0
    return x % m if isinstance(x, int) else jnp.bitwise_and(x, m - 1)


def _kernel(x_hbm, wq_hbm, k_hbm, v_hbm, wo_hbm, w3t_hbm, w4_hbm, out_ref,
            x_v, wq_v, k_v, v_v, wo_v, w3t_v, w4_v, q_v, t_v, o_v, ocol_v, s_v, vec_v,
            *, heads, window, seq, dh, d, f):
    scale = dh ** -0.5
    groups = heads // _GROUP
    half = window // 2
    n_blk = half // (_SEG * _BLOCK)
    blk_rows = 2 * _SEG * _BLOCK
    piece = _GROUP * dh // (2 * n_blk)
    first_key = seq - window
    w4_early = f - _GROUP * dh
    ring = _LO_AHEAD * _BLOCK
    all_cols = slice(None)

    pro = [((wq_hbm, wq_v, pl.ds(r, _WQ_ROWS), pl.ds(0, _WQ_HI)),
            (wq_hbm, wq_v, pl.ds(r, _WQ_ROWS), pl.ds(_WQ_HI, heads * dh - _WQ_HI)))
           for r in range(0, d, _WQ_ROWS)]
    n_wq = len(pro)
    for src, dst, total in ((w3t_hbm, w3t_v, f), (w4_hbm, w4_v, w4_early)):
        for r in range(0, total, _W_ROWS):
            n = min(_W_ROWS, total - r)
            if n > _W_HI:
                pro.append(((src, dst, pl.ds(r, _W_HI), all_cols),
                            (src, dst, pl.ds(r + _W_HI, n - _W_HI), all_cols)))
            else:
                pro.append((None, (src, dst, pl.ds(r, n), all_cols)))
    n_pro = len(pro)
    vpu_row0 = (_GROUP - 1) * dh
    tail = [(h * dh, dh) for h in range(_GROUP - 1)]
    tail += [(r, _VPU_ROWS) for r in range(vpu_row0, vpu_row0 + dh, _VPU_ROWS)]

    def body(sem_x, sem_pro_hi, sem_pro_lo, sem_hi, sem_lo, sem_piece, sem_tail):
        def block_copy(spec, sem):
            src, dst, rows, cols = spec
            return pltpu.make_async_copy(src.at[rows, cols], dst.at[rows, cols], sem)

        def pro_start(i):
            hi, lo = pro[i]
            if hi is not None:
                block_copy(hi, sem_pro_hi.at[i]).start(priority=_HI)
            block_copy(lo, sem_pro_lo.at[i]).start(priority=_LO)

        def pro_wait(i):
            hi, lo = pro[i]
            if hi is not None:
                block_copy(hi, sem_pro_hi.at[i]).wait()
            block_copy(lo, sem_pro_lo.at[i]).wait()

        def kv_copy(g, phase, j, lo):
            src, dst = (k_hbm, k_v) if phase == 0 else (v_hbm, v_v)
            key = _aligned(first_key + (half if lo else 0) + j * _SEG, _SEG)
            row = _aligned(2 * _SEG * j + (_SEG if lo else 0), _SEG)
            sem = (sem_lo if lo else sem_hi).at[_mod_pow2(j, ring)]
            return pltpu.make_async_copy(
                src.at[0, pl.ds(g * _GROUP, _GROUP), pl.ds(key, _SEG), :],
                dst.at[_mod_pow2(g, 2), :, pl.ds(row, _SEG), :], sem)

        def piece_copy(g, phase, b):
            i = phase * n_blk + b
            sem = sem_piece.at[_mod_pow2(i, _HI_AHEAD)]
            if isinstance(g, int) and g == 0:
                rows = pl.ds(_aligned(w4_early + i * piece, piece), piece)
                return block_copy((w4_hbm, w4_v, rows, all_cols), sem)
            rows = pl.ds(_aligned(g * _GROUP * dh + i * piece, piece), piece)
            return block_copy((wo_hbm, wo_v, rows, all_cols), sem)

        def tail_copy(i):
            return block_copy((wo_hbm, wo_v, pl.ds(*tail[i]), all_cols), sem_tail.at[i])

        x_copy = pltpu.make_async_copy(x_hbm, x_v, sem_x.at[0])
        x_copy.start()
        for i in range(_PRO_AHEAD):
            pro_start(i)
        x_copy.wait()
        x = jnp.broadcast_to(x_v[0].astype(_F32), (_ROWS, d))
        xn = _layernorm(x)
        xn_b = xn.astype(_BF16)
        vec_v[0] = x
        vec_v[1] = xn
        vec_v[2] = jnp.zeros((_ROWS, d), _F32)

        q = None
        per_step = n_wq // _Q_STEPS
        n_hi, n_lo = _HI_AHEAD * _BLOCK, _LO_AHEAD * _BLOCK
        for i in range(n_pro):
            pro_wait(i)
            if i + _PRO_AHEAD < n_pro:
                pro_start(i + _PRO_AHEAD)
            else:
                k = i + _PRO_AHEAD - n_pro
                for e in range(k * n_hi // _PRO_AHEAD, (k + 1) * n_hi // _PRO_AHEAD):
                    if e % _BLOCK == 0:
                        piece_copy(0, 0, e // _BLOCK).start(priority=_HI)
                    kv_copy(0, 0, e, False).start(priority=_HI)
                for e in range(k * n_lo // _PRO_AHEAD, (k + 1) * n_lo // _PRO_AHEAD):
                    kv_copy(0, 0, e, True).start(priority=_LO)
            if i < n_wq and (i + 1) % per_step == 0:
                r1 = (i + 1) * _WQ_ROWS
                r0 = r1 - per_step * _WQ_ROWS
                part = jnp.dot(xn_b[:, r0:r1], wq_v[r0:r1, :], preferred_element_type=_F32)
                q = part if q is None else q + part
                if i == n_wq - 1:
                    for h in range(heads):
                        q_v[h] = q[:, h * dh:(h + 1) * dh].astype(_BF16)
        hidden = jax.lax.dot_general(_layernorm(xn).astype(_BF16), w3t_v[...], _NT,
                                     preferred_element_type=_F32)
        t_v[...] = jax.nn.gelu(hidden, approximate=True).astype(_BF16)

        def ahead(phase, b0, n):
            dg, t = divmod(phase * n_blk + b0 + n, 2 * n_blk)
            ph, b = divmod(t, n_blk)
            return dg, ph, b - b0

        def segment(g, phase, b0, carry, compute):
            last = isinstance(g, int) and g == groups - 1
            g_hi, ph_hi, b_hi = ahead(phase, b0, _HI_AHEAD)
            g_lo, ph_lo, b_lo = ahead(phase, b0, _LO_AHEAD)
            start_hi = not (last and g_hi > 0)
            start_lo = not (last and g_lo > 0)

            def block(b, carry):
                piece_copy(g, phase, b).wait()
                for t in range(_BLOCK):
                    j = b * _BLOCK + t
                    kv_copy(g, phase, j, False).wait()
                    kv_copy(g, phase, j, True).wait()
                    if start_hi:
                        if t == _BLOCK - 1:
                            piece_copy(g + g_hi, ph_hi, b + b_hi).start(priority=_HI)
                        kv_copy(g + g_hi, ph_hi, j + b_hi * _BLOCK, False).start(priority=_HI)
                    if start_lo:
                        kv_copy(g + g_lo, ph_lo, j + b_lo * _BLOCK, True).start(priority=_LO)
                return compute(b, carry)

            return jax.lax.fori_loop(b0, b0 + _HI_AHEAD, block, carry)

        def group(g):
            slot = _mod_pow2(g, 2)
            members = range(_GROUP)

            def keys(ref, i, b):
                return ref[slot, i, pl.ds(pl.multiple_of(b * blk_rows, blk_rows), blk_rows), :]

            def qk(b, m):
                out = []
                for i in members:
                    s = jax.lax.dot_general(q_v[g * _GROUP + i], keys(k_v, i, b), _NT,
                                            preferred_element_type=_F32)
                    s_v[i, b] = s
                    out.append(jnp.maximum(m[i], s))
                return tuple(out)

            m = tuple(jnp.full((_ROWS, blk_rows), -jnp.inf, _F32) for _ in members)
            for b0 in range(0, n_blk, _HI_AHEAD):
                m = segment(g, 0, b0, m, qk)
            m = [jnp.max(mi, axis=-1, keepdims=True) for mi in m]

            def pv(b, carry):
                l, o = carry
                l_out, o_out = [], []
                for i in members:
                    p = jnp.exp((s_v[i, b] - m[i]) * scale)
                    l_out.append(l[i] + p)
                    o_out.append(o[i] + jnp.dot(p.astype(_BF16), keys(v_v, i, b),
                                                preferred_element_type=_F32))
                return tuple(l_out), tuple(o_out)

            carry = (tuple(jnp.zeros((_ROWS, blk_rows), _F32) for _ in members),
                     tuple(jnp.zeros((_ROWS, dh), _F32) for _ in members))
            for b0 in range(0, n_blk, _HI_AHEAD):
                if (isinstance(g, int) and g == groups - 1
                        and b0 == n_blk - _LO_AHEAD):
                    for i in range(len(tail)):
                        tail_copy(i).start(priority=_LO)
                carry = segment(g, 1, b0, carry, pv)
            l, o = carry
            o = [(o[i] / jnp.sum(l[i], axis=-1, keepdims=True)).astype(_BF16) for i in members]
            if isinstance(g, int) and g == 0:
                for i in range(_GROUP - 1):
                    o_v[i] = o[i]
                ocol_v[...] = jnp.broadcast_to(o[-1][0:1].astype(_F32), (dh, dh)).T
                z = vec_v[1] + jnp.dot(t_v[...], w4_v[...], preferred_element_type=_F32)
                vec_v[3] = z * jax.nn.sigmoid(z)
            else:
                rows = pl.ds(_aligned(g * _GROUP * dh, _GROUP * dh), _GROUP * dh)
                vec_v[2] += jnp.dot(jnp.concatenate(o, axis=1), wo_v[rows, :],
                                    preferred_element_type=_F32)

        group(0)

        def loop_group(g, carry):
            group(g)
            return carry

        jax.lax.fori_loop(1, groups - 1, loop_group, 0)
        group(groups - 1)

        s = vec_v[2]
        partial = jnp.zeros((_ROWS, d), _F32)
        for i, (r0, n) in enumerate(tail):
            tail_copy(i).wait()
            if r0 < vpu_row0:
                s = s + jnp.dot(o_v[i], wo_v[r0:r0 + n, :], preferred_element_type=_F32)
            else:
                w = wo_v[r0:r0 + n, :].astype(_F32)
                for r in range(0, n, _ROWS):
                    col = ocol_v[pl.ds(r0 - vpu_row0 + r, _ROWS), :]
                    col = jnp.concatenate([col] * (d // dh), axis=1)
                    partial = partial + w[r:r + _ROWS, :] * col
        s = s[0:1] + jnp.sum(partial, axis=0, keepdims=True)
        out = vec_v[0][0:1] + s * vec_v[3][0:1]
        out_ref[0] = out.astype(out_ref.dtype)

    dma = pltpu.SemaphoreType.DMA
    pl.run_scoped(body, dma((1,)), dma((n_pro,)), dma((n_pro,)), dma((ring,)), dma((ring,)),
                  dma((_HI_AHEAD,)), dma((len(tail),)))


@jax.jit
def pallas_recurrent_scan__sliding_block_cached__mixer_s_mlp__decode_kernel(
    A_x, A_k_cache, A_v_cache, A_wq, A_wo, B_x, B_w1, B_w2, B_w3, B_w4,
):
    b, sq, d = A_x.shape
    _, heads, seq, dh = A_k_cache.shape
    f = B_w3.shape[1]
    window = min(4096, max(256, seq // 4))
    blk_rows = 2 * _SEG * _BLOCK
    n_blk = window // blk_rows
    assert b == 1 and sq == 1 and A_wq.shape[1] == heads * dh
    assert heads % _GROUP == 0 and heads // _GROUP >= 2 and d % dh == 0 and f % 16 == 0
    assert window % blk_rows == 0 and n_blk % _LO_AHEAD == 0 and _LO_AHEAD % _HI_AHEAD == 0

    return pl.pallas_call(
        functools.partial(_kernel, heads=heads, window=window, seq=seq, dh=dh, d=d, f=f),
        in_specs=[pl.BlockSpec(memory_space=pl.ANY)] * 7,
        out_specs=pl.BlockSpec(memory_space=pltpu.VMEM),
        out_shape=jax.ShapeDtypeStruct((b, sq, d), A_x.dtype),
        scratch_shapes=[
            pltpu.VMEM((1, 1, d), _BF16),
            pltpu.VMEM((d, heads * dh), _BF16),
            pltpu.VMEM((2, _GROUP, window, dh), _BF16),
            pltpu.VMEM((2, _GROUP, window, dh), _BF16),
            pltpu.VMEM((heads * dh, d), _BF16),
            pltpu.VMEM((f, d), _BF16),
            pltpu.VMEM((f, d), _BF16),
            pltpu.VMEM((heads, _ROWS, dh), _BF16),
            pltpu.VMEM((_ROWS, f), _BF16),
            pltpu.VMEM((_GROUP - 1, _ROWS, dh), _BF16),
            pltpu.VMEM((dh, dh), _F32),
            pltpu.VMEM((_GROUP, n_blk, _ROWS, blk_rows), _F32),
            pltpu.VMEM((4, _ROWS, d), _F32),
        ],
        compiler_params=pltpu.CompilerParams(
            vmem_limit_bytes=48 * 1024 * 1024,
            disable_bounds_checks=True,
        ),
    )(A_x, A_wq, A_k_cache, A_v_cache, A_wo, B_w3.T, B_w4)
```

```python
import functools

import jax
import jax.numpy as jnp
import jax.experimental.pallas as pl
import jax.experimental.pallas.tpu as pltpu

_EPS = 1e-5
_F32 = jnp.float32
_BF16 = jnp.bfloat16
_NT = (((1,), (1,)), ((), ()))

_ROWS = 8
_GROUP = 4
_SEG = 16
_BLOCK = 8
_LO_AHEAD = 8
_HI_AHEAD = 4
_WQ_ROWS = 8
_WQ_HI = 1024
_PRO_AHEAD = 32
_Q_STEPS = 4
_VPU_ROWS = 64
_HI, _LO = 0, 1


def _layernorm(x):
    m = jnp.mean(x, axis=-1, keepdims=True)
    xc = x - m
    v = jnp.mean(xc * xc, axis=-1, keepdims=True)
    return xc / jnp.sqrt(v + _EPS)


def _aligned(x, m):
    return x if isinstance(x, int) else pl.multiple_of(x, m)


def _mod_pow2(x, m):
    assert m & (m - 1) == 0
    return x % m if isinstance(x, int) else jnp.bitwise_and(x, m - 1)


def _kernel(x_hbm, wq_hbm, k_hbm, v_hbm, wo_hbm, w3t_hbm, w4_hbm, out_ref,
            x_v, wq_v, k_v, v_v, wo_v, w3t_v, w4_v, q_v, t_v, o_v, ocol_v, s_v, vec_v,
            *, heads, window, seq, dh, d, f):
    scale = dh ** -0.5
    groups = heads // _GROUP
    half = window // 2
    n_blk = half // (_SEG * _BLOCK)
    blk_rows = 2 * _SEG * _BLOCK
    piece = _GROUP * dh // (2 * n_blk)
    first_key = seq - window
    w4_early = f - _GROUP * dh
    ring = _LO_AHEAD * _BLOCK
    all_cols = slice(None)

    pro = [((wq_hbm, wq_v, pl.ds(r, _WQ_ROWS), pl.ds(0, _WQ_HI)),
            (wq_hbm, wq_v, pl.ds(r, _WQ_ROWS), pl.ds(_WQ_HI, heads * dh - _WQ_HI)))
           for r in range(0, d, _WQ_ROWS)]
    n_pro = len(pro)
    extras, g0 = [], 1
    for src, dst, rows in ((w3t_hbm, w3t_v, f), (w4_hbm, w4_v, w4_early)):
        assert rows % piece == 0
        extras.append((src, dst, g0, rows // piece))
        g0 += pl.cdiv(rows // piece, 2 * n_blk)
    assert g0 < groups
    vpu_row0 = (_GROUP - 1) * dh
    tail = [(h * dh, dh) for h in range(_GROUP - 1)]
    tail += [(r, _VPU_ROWS) for r in range(vpu_row0, vpu_row0 + dh, _VPU_ROWS)]

    def body(sem_x, sem_pro_hi, sem_pro_lo, sem_hi, sem_lo, sem_piece, sem_extra, sem_tail):
        def block_copy(spec, sem):
            src, dst, rows, cols = spec
            return pltpu.make_async_copy(src.at[rows, cols], dst.at[rows, cols], sem)

        def pro_start(i):
            block_copy(pro[i][0], sem_pro_hi.at[i]).start(priority=_HI)
            block_copy(pro[i][1], sem_pro_lo.at[i]).start(priority=_LO)

        def pro_wait(i):
            block_copy(pro[i][0], sem_pro_hi.at[i]).wait()
            block_copy(pro[i][1], sem_pro_lo.at[i]).wait()

        def kv_copy(g, phase, j, lo):
            src, dst = (k_hbm, k_v) if phase == 0 else (v_hbm, v_v)
            key = _aligned(first_key + (half if lo else 0) + j * _SEG, _SEG)
            row = _aligned(2 * _SEG * j + (_SEG if lo else 0), _SEG)
            sem = (sem_lo if lo else sem_hi).at[_mod_pow2(j, ring)]
            return pltpu.make_async_copy(
                src.at[0, pl.ds(g * _GROUP, _GROUP), pl.ds(key, _SEG), :],
                dst.at[_mod_pow2(g, 2), :, pl.ds(row, _SEG), :], sem)

        def piece_copy(g, phase, b):
            i = phase * n_blk + b
            sem = sem_piece.at[_mod_pow2(i, _HI_AHEAD)]
            if isinstance(g, int) and g == 0:
                rows = pl.ds(_aligned(w4_early + i * piece, piece), piece)
                return block_copy((w4_hbm, w4_v, rows, all_cols), sem)
            rows = pl.ds(_aligned(g * _GROUP * dh + i * piece, piece), piece)
            return block_copy((wo_hbm, wo_v, rows, all_cols), sem)

        def for_extra_copy(g, phase, b, act):
            i = phase * n_blk + b
            sem = sem_extra.at[_mod_pow2(i, _HI_AHEAD)]
            for src, dst, first, n in extras:
                if isinstance(g, int) and not 0 <= (g - first) * 2 * n_blk < n:
                    continue
                k = (g - first) * 2 * n_blk + i

                def run(src=src, dst=dst, k=k, n=n):
                    k = k if isinstance(k, int) else jnp.clip(k, 0, n - 1)
                    rows = pl.ds(_aligned(k * piece, piece), piece)
                    act(block_copy((src, dst, rows, all_cols), sem))

                if isinstance(k, int):
                    if 0 <= k < n:
                        run()
                else:
                    pl.when(jnp.logical_and(k >= 0, k < n))(run)

        def tail_copy(i):
            return block_copy((wo_hbm, wo_v, pl.ds(*tail[i]), all_cols), sem_tail.at[i])

        x_copy = pltpu.make_async_copy(x_hbm, x_v, sem_x.at[0])
        x_copy.start()
        for i in range(_PRO_AHEAD):
            pro_start(i)
        x_copy.wait()
        x = jnp.broadcast_to(x_v[0].astype(_F32), (_ROWS, d))
        xn = _layernorm(x)
        xn_b = xn.astype(_BF16)
        vec_v[0] = x
        vec_v[1] = xn
        vec_v[2] = jnp.zeros((_ROWS, d), _F32)

        q = None
        per_step = n_pro // _Q_STEPS
        n_hi, n_lo = _HI_AHEAD * _BLOCK, _LO_AHEAD * _BLOCK
        for i in range(n_pro):
            pro_wait(i)
            if i + _PRO_AHEAD < n_pro:
                pro_start(i + _PRO_AHEAD)
            else:
                k = i + _PRO_AHEAD - n_pro
                for e in range(k * n_hi // _PRO_AHEAD, (k + 1) * n_hi // _PRO_AHEAD):
                    if e % _BLOCK == 0:
                        piece_copy(0, 0, e // _BLOCK).start(priority=_HI)
                    kv_copy(0, 0, e, False).start(priority=_HI)
                for e in range(k * n_lo // _PRO_AHEAD, (k + 1) * n_lo // _PRO_AHEAD):
                    kv_copy(0, 0, e, True).start(priority=_LO)
            if (i + 1) % per_step == 0:
                r1 = (i + 1) * _WQ_ROWS
                r0 = r1 - per_step * _WQ_ROWS
                part = jnp.dot(xn_b[:, r0:r1], wq_v[r0:r1, :], preferred_element_type=_F32)
                q = part if q is None else q + part
        for h in range(heads):
            q_v[h] = q[:, h * dh:(h + 1) * dh].astype(_BF16)

        def mlp_hidden():
            hidden = jax.lax.dot_general(_layernorm(vec_v[1]).astype(_BF16), w3t_v[...], _NT,
                                         preferred_element_type=_F32)
            t_v[...] = jax.nn.gelu(hidden, approximate=True).astype(_BF16)

        def mlp_gate():
            z = vec_v[1] + jnp.dot(t_v[...], w4_v[...], preferred_element_type=_F32)
            vec_v[3] = z * jax.nn.sigmoid(z)

        def ahead(phase, b0, n):
            dg, t = divmod(phase * n_blk + b0 + n, 2 * n_blk)
            ph, b = divmod(t, n_blk)
            return dg, ph, b - b0

        def segment(g, phase, b0, carry, compute):
            last = isinstance(g, int) and g == groups - 1
            g_hi, ph_hi, b_hi = ahead(phase, b0, _HI_AHEAD)
            g_lo, ph_lo, b_lo = ahead(phase, b0, _LO_AHEAD)
            start_hi = not (last and g_hi > 0)
            start_lo = not (last and g_lo > 0)

            def block(b, carry):
                piece_copy(g, phase, b).wait()
                for_extra_copy(g, phase, b, lambda cp: cp.wait())
                for t in range(_BLOCK):
                    j = b * _BLOCK + t
                    kv_copy(g, phase, j, False).wait()
                    kv_copy(g, phase, j, True).wait()
                    if start_hi:
                        if t == _BLOCK // 2 - 1:
                            for_extra_copy(g + g_hi, ph_hi, b + b_hi,
                                           lambda cp: cp.start(priority=_HI))
                        if t == _BLOCK - 1:
                            piece_copy(g + g_hi, ph_hi, b + b_hi).start(priority=_HI)
                        kv_copy(g + g_hi, ph_hi, j + b_hi * _BLOCK, False).start(priority=_HI)
                    if start_lo:
                        kv_copy(g + g_lo, ph_lo, j + b_lo * _BLOCK, True).start(priority=_LO)
                return compute(b, carry)

            return jax.lax.fori_loop(b0, b0 + _HI_AHEAD, block, carry)

        def group(g):
            slot = _mod_pow2(g, 2)
            members = range(_GROUP)
            last = isinstance(g, int) and g == groups - 1

            def keys(ref, i, b):
                return ref[slot, i, pl.ds(pl.multiple_of(b * blk_rows, blk_rows), blk_rows), :]

            def qk(b, m):
                out = []
                for i in members:
                    s = jax.lax.dot_general(q_v[g * _GROUP + i], keys(k_v, i, b), _NT,
                                            preferred_element_type=_F32)
                    s_v[i, b] = s
                    out.append(jnp.maximum(m[i], s))
                return tuple(out)

            m = tuple(jnp.full((_ROWS, blk_rows), -jnp.inf, _F32) for _ in members)
            for b0 in range(0, n_blk, _HI_AHEAD):
                if last and b0 == _HI_AHEAD:
                    mlp_hidden()
                if last and b0 == 2 * _HI_AHEAD:
                    mlp_gate()
                m = segment(g, 0, b0, m, qk)
            m = [jnp.max(mi, axis=-1, keepdims=True) for mi in m]

            def pv(b, carry):
                l, o = carry
                l_out, o_out = [], []
                for i in members:
                    p = jnp.exp((s_v[i, b] - m[i]) * scale)
                    l_out.append(l[i] + p)
                    o_out.append(o[i] + jnp.dot(p.astype(_BF16), keys(v_v, i, b),
                                                preferred_element_type=_F32))
                return tuple(l_out), tuple(o_out)

            carry = (tuple(jnp.zeros((_ROWS, blk_rows), _F32) for _ in members),
                     tuple(jnp.zeros((_ROWS, dh), _F32) for _ in members))
            for b0 in range(0, n_blk, _HI_AHEAD):
                if last and b0 == n_blk - _LO_AHEAD:
                    for i in range(len(tail)):
                        tail_copy(i).start(priority=_LO)
                carry = segment(g, 1, b0, carry, pv)
            l, o = carry
            o = [(o[i] / jnp.sum(l[i], axis=-1, keepdims=True)).astype(_BF16) for i in members]
            if isinstance(g, int) and g == 0:
                for i in range(_GROUP - 1):
                    o_v[i] = o[i]
                ocol_v[...] = jnp.broadcast_to(o[-1][0:1].astype(_F32), (dh, dh)).T
            else:
                rows = pl.ds(_aligned(g * _GROUP * dh, _GROUP * dh), _GROUP * dh)
                vec_v[2] += jnp.dot(jnp.concatenate(o, axis=1), wo_v[rows, :],
                                    preferred_element_type=_F32)

        group(0)

        def loop_group(g, carry):
            group(g)
            return carry

        jax.lax.fori_loop(1, groups - 1, loop_group, 0)
        group(groups - 1)

        s = vec_v[2]
        partial = jnp.zeros((_ROWS, d), _F32)
        for i, (r0, n) in enumerate(tail):
            tail_copy(i).wait()
            if r0 < vpu_row0:
                s = s + jnp.dot(o_v[i], wo_v[r0:r0 + n, :], preferred_element_type=_F32)
            else:
                w = wo_v[r0:r0 + n, :].astype(_F32)
                for r in range(0, n, _ROWS):
                    col = ocol_v[pl.ds(r0 - vpu_row0 + r, _ROWS), :]
                    col = jnp.concatenate([col] * (d // dh), axis=1)
                    partial = partial + w[r:r + _ROWS, :] * col
        s = s[0:1] + jnp.sum(partial, axis=0, keepdims=True)
        out = vec_v[0][0:1] + s * vec_v[3][0:1]
        out_ref[0] = out.astype(out_ref.dtype)

    dma = pltpu.SemaphoreType.DMA
    pl.run_scoped(body, dma((1,)), dma((n_pro,)), dma((n_pro,)), dma((ring,)), dma((ring,)),
                  dma((_HI_AHEAD,)), dma((_HI_AHEAD,)), dma((len(tail),)))


@jax.jit
def pallas_recurrent_scan__sliding_block_cached__mixer_s_mlp__decode_kernel(
    A_x, A_k_cache, A_v_cache, A_wq, A_wo, B_x, B_w1, B_w2, B_w3, B_w4,
):
    b, sq, d = A_x.shape
    _, heads, seq, dh = A_k_cache.shape
    f = B_w3.shape[1]
    window = min(4096, max(256, seq // 4))
    blk_rows = 2 * _SEG * _BLOCK
    n_blk = window // blk_rows
    assert b == 1 and sq == 1 and A_wq.shape[1] == heads * dh
    assert heads % _GROUP == 0 and heads // _GROUP >= 2 and d % dh == 0 and f % 16 == 0
    assert window % blk_rows == 0 and n_blk % _LO_AHEAD == 0 and _LO_AHEAD % _HI_AHEAD == 0
    assert n_blk >= 3 * _HI_AHEAD

    return pl.pallas_call(
        functools.partial(_kernel, heads=heads, window=window, seq=seq, dh=dh, d=d, f=f),
        in_specs=[pl.BlockSpec(memory_space=pl.ANY)] * 7,
        out_specs=pl.BlockSpec(memory_space=pltpu.VMEM),
        out_shape=jax.ShapeDtypeStruct((b, sq, d), A_x.dtype),
        scratch_shapes=[
            pltpu.VMEM((1, 1, d), _BF16),
            pltpu.VMEM((d, heads * dh), _BF16),
            pltpu.VMEM((2, _GROUP, window, dh), _BF16),
            pltpu.VMEM((2, _GROUP, window, dh), _BF16),
            pltpu.VMEM((heads * dh, d), _BF16),
            pltpu.VMEM((f, d), _BF16),
            pltpu.VMEM((f, d), _BF16),
            pltpu.VMEM((heads, _ROWS, dh), _BF16),
            pltpu.VMEM((_ROWS, f), _BF16),
            pltpu.VMEM((_GROUP - 1, _ROWS, dh), _BF16),
            pltpu.VMEM((dh, dh), _F32),
            pltpu.VMEM((_GROUP, n_blk, _ROWS, blk_rows), _F32),
            pltpu.VMEM((4, _ROWS, d), _F32),
        ],
        compiler_params=pltpu.CompilerParams(
            vmem_limit_bytes=48 * 1024 * 1024,
            disable_bounds_checks=True,
        ),
    )(A_x, A_wq, A_k_cache, A_v_cache, A_wo, B_w3.T, B_w4)
```
